```python
import os as _os
_os.environ.setdefault("JAX_PLATFORMS", "cpu")
import jax
import jax.numpy as jnp

def _softmax(x, axis=-1):
    return jax.nn.softmax(x, axis=axis)
def _gelu(x):
    return jax.nn.gelu(x, approximate=True)
def _silu(x):
    return jax.nn.silu(x)
def _sigmoid(x):
    return jax.nn.sigmoid(x)
def _layernorm(x, axis=-1, eps=1e-5):
    m = jnp.mean(x, axis=axis, keepdims=True)
    v = jnp.var(x, axis=axis, keepdims=True)
    return (x - m) / jnp.sqrt(v + eps)
def _scatter_add(tgt, idx, src, axis=0):
    return tgt.at[idx].add(src)
def _segment_sum(src, seg, n):
    return jax.ops.segment_sum(src, seg, n)
class _Rng:
    def __init__(self, key):
        self._k = key
    def _next(self):
        self._k, sub = jax.random.split(self._k)
        return sub
    def normal(self, shape):
        return jax.random.normal(self._next(), shape, dtype=jnp.bfloat16)
    def randint(self, lo, hi, shape):
        return jax.random.randint(self._next(), shape, lo, hi, dtype=jnp.int32)
    def uniform(self, shape, lo=0.0, hi=1.0):
        return jax.random.uniform(self._next(), shape, jnp.bfloat16, lo, hi)
    def permutation(self, n):
        return jax.random.permutation(self._next(), n)


kernel_name = 'concat_heads__sliding_block__ssm_conv_s4__prompt'

def setup_inputs():
    _rng = _Rng(jax.random.key(int.from_bytes(__import__("os").urandom(4), "little")))
    _w = (lambda a: (lambda t: t.astype(jnp.bfloat16) if jnp.issubdtype(t.dtype, jnp.floating) else t)(jnp.asarray(a)))
    def _A_setup():
        B, S, D = 1, 2048, 512
        return {
            "x": _w((lambda *s: _rng.normal(s) * 0.2)(B, S, D)),
            "wqkv": _w((lambda *s: _rng.normal(s) * 0.2)(D, 3 * D)),
            "wo": _w((lambda *s: _rng.normal(s) * 0.05)(D, D)),
        }
    _A_in = _A_setup()

    def _B_setup():
        B, L, D, N = 1, 2048, 512, 128
        A_re = -jnp.exp((lambda *s: _rng.normal(s) * 0.8)(D, N))
        A_im = jnp.pi * (lambda *s: _rng.normal(s) * 0.8)(D, N)
        B_re = (lambda *s: _rng.normal(s) * 0.8)(D, N)
        B_im = (lambda *s: _rng.normal(s) * 0.8)(D, N)
        C_re = (lambda *s: _rng.normal(s) * 0.8)(D, N)
        C_im = (lambda *s: _rng.normal(s) * 0.8)(D, N)
        log_dt = (lambda *s: _rng.normal(s) * 0.8)(D) * 0.5 - 4.0
        Dskip = (lambda *s: _rng.normal(s) * 0.05)(D)
        return {
            "u": _w((lambda *s: _rng.normal(s) * 0.05)(B, L, D)),
            "A_re": _w(A_re),
            "A_im": _w(A_im),
            "B_re": _w(B_re),
            "B_im": _w(B_im),
            "C_re": _w(C_re),
            "C_im": _w(C_im),
            "log_dt": _w(log_dt),
            "Dskip": _w(Dskip),
        }
    _B_in = _B_setup()

    return {
        "A_x": _A_in["x"],
        "A_wqkv": _A_in["wqkv"],
        "A_wo": _A_in["wo"],
        "B_u": _B_in["u"],
        "B_A_re": _B_in["A_re"],
        "B_A_im": _B_in["A_im"],
        "B_B_re": _B_in["B_re"],
        "B_B_im": _B_in["B_im"],
        "B_C_re": _B_in["C_re"],
        "B_C_im": _B_in["C_im"],
        "B_log_dt": _B_in["log_dt"],
        "B_Dskip": _B_in["Dskip"],
    }

def reference(A_x, A_wqkv, A_wo, B_u, B_A_re, B_A_im, B_B_re, B_B_im, B_C_re, B_C_im, B_log_dt, B_Dskip):
    def _A_ref(x, wqkv, wo):
        B, S, D = x.shape
        H = 32; Dh = D // H; W = 256
        qkv = (lambda x, *d: x.transpose(*d))((x @ wqkv).reshape(B, S, 3, H, Dh), 2, 0, 3, 1, 4)
        q, k, v = qkv[0], qkv[1], qkv[2]
        scores = jnp.einsum("bhqd,bhkd->bhqk", q, k) * (Dh ** -0.5)
        idx = jnp.arange(S)
        mask = (idx[:, None] - idx[None, :] >= 0) & (idx[:, None] - idx[None, :] < W)
        scores = jnp.where(mask[None, None], scores, -1e9)
        p = _softmax(scores, axis=-1)
        o = jnp.einsum("bhqk,bhkd->bhqd", p, v)
        return (lambda x, *d: x.transpose(*d))(o, 0, 2, 1, 3).reshape(B, S, D) @ wo

    def _B_ref(u, A_re, A_im, B_re, B_im, C_re, C_im, log_dt, Dskip):
        Bsz, L, D = u.shape
        dt = jnp.exp(log_dt)[:, None]
        A = A_re + 1j * A_im
        Bc = B_re + 1j * B_im
        Cc = C_re + 1j * C_im
        logdA = dt * A
        dB = dt * Bc
        l = (lambda x, dt: x.astype(dt))(jnp.arange(L), A_re.dtype)
        P = jnp.exp(logdA[:, :, None] * l[None, None, :])
        K = jnp.einsum("dn,dnl,dn->dl", Cc, P, dB).real
        L2 = 2 * L
        Kp = jnp.pad(K, ((0, 0), (0, L)))
        up = (lambda x, *d: x.transpose(*d))(u, 0, 2, 1)
        up = jnp.pad(up, ((0, 0), (0, 0), (0, L)))
        Kf = (lambda x, axes=(-2,-1): jnp.fft.rfft2(x.astype(jnp.float32), axes=axes))(Kp[:, None, :], axes=(-2, -1))
        Uf = (lambda x, axes=(-2,-1): jnp.fft.rfft2(x.astype(jnp.float32), axes=axes))(up[:, :, None, :], axes=(-2, -1))
        Yf = Uf * Kf[None, :, :, :]
        y = (lambda x, s, axes=(-2,-1): jnp.fft.irfft2(x, s=s, axes=axes).astype(jnp.bfloat16))(Yf, (1, L2), axes=(-2, -1))[:, :, 0, :L]
        y = (lambda x, *d: x.transpose(*d))(y, 0, 2, 1) + u * Dskip[None, None, :]
        return y

    a = _A_ref(A_x, A_wqkv, A_wo)
    b = _B_ref(B_u, B_A_re, B_A_im, B_B_re, B_B_im, B_C_re, B_C_im, B_log_dt, B_Dskip)
    return jnp.concatenate([a, b], axis=-1)
```

```python
import functools
import math

import numpy as np
import jax
import jax.numpy as jnp
from jax import lax
import jax.experimental.pallas as pl
import jax.experimental.pallas.tpu as pltpu

f32 = jnp.float32
bf16 = jnp.bfloat16
i32 = jnp.int32

S_LEN = 2048
D_MODEL = 512
N_HEADS = 32
D_HEAD = 16
WINDOW = 256
QB = 128
NQB = S_LEN // QB
NG = 4
NEG = -1e9
PH = 'all'


def _dot(a, b):
    return jnp.dot(a, b, preferred_element_type=f32)


def _dot_nt(a, b):
    return lax.dot_general(a, b, (((1,), (1,)), ((), ())), preferred_element_type=f32)


def _dot_tn(a, b):
    return lax.dot_general(a, b, (((0,), (0,)), ((), ())), preferred_element_type=f32)


def _attention_part(x_ref, wqkv_ref, wo_ref, out_ref, wqT, wvT, k3, qT3, vT3, oT, bias):
    for (col0, dst) in ((0, wqT), (2 * D_MODEL, wvT)):
        for r in range(4):
            for c in range(4):
                blk = wqkv_ref[pl.ds(128 * r, 128), pl.ds(col0 + 128 * c, 128)].astype(f32)
                dst[pl.ds(128 * c, 128), pl.ds(128 * r, 128)] = blk.T.astype(bf16)

    rr = lax.broadcasted_iota(i32, (QB, QB), 0)
    cc = lax.broadcasted_iota(i32, (QB, QB), 1)
    bias[0] = jnp.where(rr > cc, 0.0, NEG).astype(f32)
    bias[1] = jnp.where(rr <= cc, 0.0, NEG).astype(f32)

    wk = wqkv_ref[:, pl.ds(D_MODEL, D_MODEL)]

    def proj_body(i, c):
        r0 = pl.multiple_of(i * QB, QB)
        xb = x_ref[pl.ds(r0, QB), :]
        kb = _dot(xb, wk).astype(bf16)
        for g in range(NG):
            k3[g, pl.ds(r0, QB), :] = kb[:, 128 * g:128 * (g + 1)]
        qT3[i] = (_dot_nt(wqT[...], xb) * (D_HEAD ** -0.5 * math.log2(math.e))).astype(bf16)
        vT3[i] = _dot_nt(wvT[...], xb).astype(bf16)
        return c

    lax.fori_loop(0, NQB, proj_body, 0)

    def scores(i, nblk, h):
        g, hh = divmod(h, 8)
        d0 = 128 * g + D_HEAD * hh
        qh = qT3[i, pl.ds(d0, D_HEAD), :]
        pieces = []
        if hh > 0:
            pieces.append(jnp.zeros((D_HEAD * hh, QB), bf16))
        pieces.append(qh)
        if hh < 7:
            pieces.append(jnp.zeros((128 - D_HEAD * (hh + 1), QB), bf16))
        qsel = jnp.concatenate(pieces, axis=0)
        s_list = []
        for j in range(nblk):
            kr0 = pl.multiple_of((i - j) * QB, QB)
            s_list.append(_dot(k3[g, pl.ds(kr0, QB), :], qsel))
        return s_list

    def finish(i, nblk, h, s_list):
        g, hh = divmod(h, 8)
        d0 = 128 * g + D_HEAD * hh
        s_list = [s + bias[1] if j == 0 else (s + bias[0] if j == 2 else s) for j, s in enumerate(s_list)]
        m = s_list[0].max(axis=0, keepdims=True)
        for s in s_list[1:]:
            m = jnp.maximum(m, s.max(axis=0, keepdims=True))
        p_list = [jnp.exp2(s - m) for s in s_list]
        l = p_list[0].sum(axis=0, keepdims=True)
        for p in p_list[1:]:
            l = l + p.sum(axis=0, keepdims=True)
        pT = jnp.concatenate(p_list[::-1], axis=0).astype(bf16)
        vTs = jnp.concatenate(
            [vT3[i - j, pl.ds(d0, D_HEAD), :] for j in range(nblk - 1, -1, -1)], axis=1)
        o = _dot(vTs, pT)
        oT[pl.ds(d0, D_HEAD), :] = (o / l).astype(bf16)

    def attend(i, nblk):
        cur = scores(i, nblk, 0)
        for h in range(N_HEADS):
            nxt = scores(i, nblk, h + 1) if h + 1 < N_HEADS else None
            finish(i, nblk, h, cur)
            cur = nxt
        r0 = pl.multiple_of(i * QB, QB)
        out_ref[pl.ds(r0, QB), pl.ds(0, D_MODEL)] = _dot_tn(oT[...], wo_ref[...]).astype(bf16)

    if PH == 'proj':
        out_ref[:, pl.ds(0, D_MODEL)] = jnp.zeros((S_LEN, D_MODEL), bf16)
        return
    attend(0, 1)
    attend(1, 2)

    def attn_body(i, c):
        attend(i, 3)
        return c

    lax.fori_loop(2, NQB, attn_body, 0)


L_SEQ = 2048
M_FFT = 4096
NJ = 66
JP = 80
PASSES2 = 3

_P1 = 1.5703125
_P2 = 4.837512969970703125e-4
_P3 = 7.54978995489188216e-8


def _sincos_poly(r):
    r2 = r * r
    s = r + r * r2 * (-1.6666654611e-1 + r2 * (8.3321608736e-3 + r2 * (-1.9515295891e-4)))
    c = 1.0 - 0.5 * r2 + r2 * r2 * (4.166664568298827e-2 + r2 * (-1.388731625493765e-3 + r2 * 2.443315711809948e-5))
    return s, c


def _quadrant_fix(q, s, c):
    swap = (q & 1) == 1
    sn = jnp.where(swap, c, s)
    cs = jnp.where(swap, s, c)
    sn = jnp.where((q & 2) == 2, -sn, sn)
    cs = jnp.where(((q + 1) & 2) == 2, -cs, cs)
    return cs, sn


def _cis(theta):
    qf = jnp.floor(theta * (2.0 / math.pi) + 0.5)
    r = theta - qf * _P1
    r = r - qf * _P2
    r = r - qf * _P3
    s, c = _sincos_poly(r)
    return _quadrant_fix(qf.astype(i32), s, c)


def _trig_int(m):
    q = (m + 512) >> 10
    r = (m - (q << 10)).astype(f32) * (2.0 * math.pi / M_FFT)
    s, c = _sincos_poly(r)
    return _quadrant_fix(q, s, c)


def _hi(x):
    return lax.bitcast_convert_type(lax.bitcast_convert_type(x, i32) & jnp.int32(-65536), f32)


def _to_packed(x_f32):
    return pltpu.bitcast(x_f32.astype(bf16), i32)


def _from_packed(x_i32):
    return pltpu.bitcast(x_i32, bf16)


def _plan_powers():
    direct = (1, 8, 64, 512)
    have, ops = set(), []

    def ensure(e):
        if e in have:
            return
        if e in direct:
            ops.append(("direct", e))
        elif e & (e - 1) == 0:
            ensure(e // 2)
            ops.append(("sq", e, e // 2))
        else:
            hb = 1 << (e.bit_length() - 1)
            ensure(hb)
            ensure(e - hb)
            ops.append(("mul", e, hb, e - hb))
        have.add(e)

    for s in (1, 2, 4, 8):
        for b in range(1, 8):
            ensure(s * b)
        for b in range(1, 8):
            ensure(8 * s * b)
    for e in (64, 128, 192, 256, 512, 1024, 2048):
        ensure(e)
    return ops


_POWER_PLAN = _plan_powers()
N_COARSE = 81
N_BLOCKS = 20


def _build_dft_tables(t1, t3, f2, f2i):
    ncol = 128 * (3 if PASSES2 == 3 else 1)
    row = lax.broadcasted_iota(i32, (128, ncol), 0)
    col = lax.broadcasted_iota(i32, (128, ncol), 1)
    p = col >> 7
    ci = col & 127
    po, k2 = row >> 6, row & 63
    pi_, n2 = ci >> 6, ci & 63
    c, s = _trig_int(((k2 * n2) & 63) << 6)
    for dst, sgn in ((f2, 1.0), (f2i, -1.0)):
        val = jnp.where(po == pi_, c, jnp.where(po == 0, sgn * s, -sgn * s))
        hi = val.astype(bf16).astype(f32)
        dst[...] = _to_packed(jnp.where(p == 1, val - hi, hi))

    def body(n2, carry):
        row = lax.broadcasted_iota(i32, (JP, 128), 0)
        col = lax.broadcasted_iota(i32, (JP, 128), 1)
        p = col >> 5
        n1 = col & 31
        k1 = row >> 1
        t = (n1 << 6) + n2
        c, s = _trig_int((k1 * t) & (M_FFT - 1))
        val = jnp.where((row & 1) == 0, c, -s)
        val = jnp.where((row < NJ) & (p < 3), val, 0.0)
        hi = val.astype(bf16).astype(f32)
        t1[n2] = _to_packed(jnp.where(p == 1, val - hi, hi))
        row = lax.broadcasted_iota(i32, (32, 256), 0)
        col = lax.broadcasted_iota(i32, (32, 256), 1)
        p = (col >= JP).astype(i32) + (col >= 2 * JP).astype(i32) + (col >= 3 * JP).astype(i32)
        j = col - JP * p
        k1 = j >> 1
        t = (row << 6) + n2
        c, s = _trig_int((k1 * t) & (M_FFT - 1))
        val = jnp.where((j & 1) == 0, c, -s)
        w = jnp.where((k1 == 0) | (k1 == 32), 1.0 / M_FFT, 2.0 / M_FFT)
        val = jnp.where((j < NJ) & (p < 3), val * w, 0.0)
        hi = val.astype(bf16).astype(f32)
        t3[n2] = _to_packed(jnp.where(p == 1, val - hi, hi))
        return carry

    lax.fori_loop(0, 64, body, 0)


def _cmul(a, b):
    return a[0] * b[0] - a[1] * b[1], a[0] * b[1] + a[1] * b[0]


def _kgen_group(g, prm_refs, ldt_ref, lam, tabF, tabC, kall):
    are, aim, bre, bim, cre, cim = prm_refs
    r0 = pl.multiple_of(g * 128, 128)
    dt = jnp.exp(ldt_ref[g].astype(f32)).astype(bf16).astype(f32)

    def tr(ref):
        return ref[pl.ds(r0, 128), :].astype(f32).T

    dbr = tr(bre) * dt
    dbi = tr(bim) * dt
    cr_, ci_ = tr(cre), tr(cim)
    lam[0] = tr(are) * dt
    lam[1] = tr(aim) * dt
    lam[2] = cr_ * dbr - ci_ * dbi
    lam[3] = cr_ * dbi + ci_ * dbr

    CH = 16

    def tab_body(ch, carry):
        rows = pl.ds(pl.multiple_of(ch * CH, CH), CH)
        lr, li = lam[0, rows, :], lam[1, rows, :]
        cc = (lam[2, rows, :], lam[3, rows, :])
        W = {}
        for op in _POWER_PLAN:
            if op[0] == "direct":
                e = float(op[1])
                mag = jnp.exp(lr * e)
                c, s = _cis(li * e)
                W[op[1]] = (mag * c, mag * s)
            elif op[0] == "sq":
                a, b = W[op[2]]
                W[op[1]] = (a * a - b * b, (a + a) * b)
            else:
                W[op[1]] = _cmul(W[op[2]], W[op[3]])
        for si, s in enumerate((1, 2, 4, 8)):
            for b in range(1, 8):
                tabF[0, 8 * si + b, rows, :] = W[s * b][0]
                tabF[1, 8 * si + b, rows, :] = W[s * b][1]

        def put(idx, v):
            tabC[0, idx, rows, :] = v[0]
            tabC[1, idx, rows, :] = v[1]

        base = cc
        for p in range(4):
            if p > 0:
                base = _cmul(cc, W[64 * p])
            put(8 * p, base)
            for i in range(1, 8):
                put(8 * p + i, _cmul(base, W[8 * i]))
        for si, s in ((1, 2), (2, 4), (3, 8)):
            base = _cmul(cc, W[128 * s])
            for p in range(2):
                if p == 1:
                    base = _cmul(base, W[64 * s])
                o = 32 + 16 * (si - 1) + 8 * p
                put(o, base)
                for i in range(1, 8):
                    put(o + i, _cmul(base, W[8 * s * i]))
        put(80, _cmul(cc, W[2048]))
        return carry

    lax.fori_loop(0, 128 // CH, tab_body, 0)

    def blk_body(kk, carry):
        si = jnp.where(kk < 8, 0, 1 + (kk - 8) // 4)
        a0 = jnp.where(kk < 8, 4 * kk, 16 + 4 * ((kk - 8) % 4))
        step = jnp.left_shift(1, si)
        fbase = 8 * si
        acc = [[None] * 8 for _ in range(4)]
        for nb in range(16):
            rows = pl.ds(8 * nb, 8)
            cr = [tabC[0, 4 * kk + a, rows, :] for a in range(4)]
            ci = [tabC[1, 4 * kk + a, rows, :] for a in range(4)]
            for b in range(8):
                if b > 0:
                    fr = tabF[0, fbase + b, rows, :]
                    fi = tabF[1, fbase + b, rows, :]
                for a in range(4):
                    term = cr[a] if b == 0 else cr[a] * fr - ci[a] * fi
                    acc[a][b] = term if nb == 0 else acc[a][b] + term
        for a in range(4):
            for b in range(8):
                row = step * (8 * (a0 + a) + b)
                kall[g, pl.ds(row, 1), :] = jnp.sum(acc[a][b], axis=0, keepdims=True)
        return carry

    lax.fori_loop(0, N_BLOCKS, blk_body, 0)
    kall[g, pl.ds(L_SEQ, 1), :] = jnp.sum(tabC[0, 80], axis=0, keepdims=True)


def _split_rhs(x, extra_zero_rows=0):
    xh = _hi(x)
    pieces = [xh, xh, x - xh]
    if extra_zero_rows:
        pieces.append(jnp.zeros((extra_zero_rows, x.shape[1]), f32))
    return jnp.concatenate(pieces, axis=0).astype(bf16)


def _round_off(n2, s):
    q = n2 // s
    rem = n2 - q * s
    up = (rem * 2 > s) | ((rem * 2 == s) & ((q & 1) == 1))
    return (q + up.astype(i32)) * s


def _ssm_part(u_ref, prm_refs, ldt_ref, dsk_ref, out_ref,
              lam, tabF, tabC, kall, uf, t1, t3, f2, f2i, bsu, bsk, zs, yp):
    _build_dft_tables(t1, t3, f2, f2i)
    for g in range(NG):
        uf[g] = u_ref[:, pl.ds(128 * g, 128)].astype(f32)

    def kg(g, c):
        _kgen_group(g, prm_refs, ldt_ref, lam, tabF, tabC, kall)
        return c

    lax.fori_loop(0, NG, kg, 0)

    def st1_body(n2, carry):
        lhs = _from_packed(t1[n2])
        o = pl.multiple_of(n2 * JP, 16)
        for g in range(NG):
            xu = uf[g, pl.ds(n2, 32, stride=64), :]
            bsu[g, pl.ds(o, JP), :] = _dot(lhs, _split_rhs(xu, 32))
            xk = jnp.concatenate([
                kall[g, pl.ds(n2, 4, stride=64), :],
                kall[g, pl.ds(256 + _round_off(n2, 2), 4, stride=64), :],
                kall[g, pl.ds(512 + _round_off(n2, 4), 8, stride=64), :],
                kall[g, pl.ds(1024 + _round_off(n2, 8), 16, stride=64), :]], axis=0)
            bsk[g, pl.ds(o, JP), :] = _dot(lhs, _split_rhs(xk, 32))
        return carry

    lax.fori_loop(0, 64, st1_body, 0)

    def prep(x):
        if PASSES2 == 3:
            return _split_rhs(x)
        return x.astype(bf16)

    def k1_body(k1, carry):
        lf = _from_packed(f2[...])
        li = _from_packed(f2i[...])
        for g in range(NG):
            X = []
            for bs in (bsu, bsk):
                b = jnp.concatenate([bs[g, pl.ds(2 * k1, 64, stride=JP), :],
                                     bs[g, pl.ds(2 * k1 + 1, 64, stride=JP), :]], axis=0)
                X.append(_dot(lf, prep(b)))
            ur, ui, kr, ki = X[0][:64], X[0][64:], X[1][:64], X[1][64:]
            y = jnp.concatenate([ur * kr - ui * ki, ur * ki + ui * kr], axis=0)
            zs[g, pl.ds(pl.multiple_of(k1 * 128, 128), 128), :] = _dot(li, prep(y))
        return carry

    lax.fori_loop(0, 33, k1_body, 0)

    def st3_body(n2, carry):
        lhs = _from_packed(t3[n2])
        for g in range(NG):
            z = jnp.concatenate([zs[g, pl.ds(n2, NJ, stride=64), :],
                                 jnp.zeros((JP - NJ, 128), f32)], axis=0)
            yp[g, pl.ds(pl.multiple_of(n2 * 32, 32), 32), :] = _dot(lhs, _split_rhs(z, 16))
        return carry

    lax.fori_loop(0, 64, st3_body, 0)

    dsk = [dsk_ref[g].astype(f32) for g in range(NG)]

    def ep_body(n1, carry):
        for q in range(4):
            r0 = pl.multiple_of(n1 * 64 + 16 * q, 16)
            for g in range(NG):
                y = jnp.concatenate([yp[g, pl.ds(32 * (16 * q) + n1, 8, stride=32), :],
                                     yp[g, pl.ds(32 * (16 * q + 8) + n1, 8, stride=32), :]], axis=0)
                yb = y.astype(bf16).astype(f32)
                ud = (uf[g, pl.ds(r0, 16), :] * dsk[g]).astype(bf16).astype(f32)
                out_ref[pl.ds(r0, 16), pl.ds(D_MODEL + 128 * g, 128)] = (yb + ud).astype(bf16)
        return carry

    lax.fori_loop(0, 32, ep_body, 0)


_SSM_SCRATCH = [
    pltpu.VMEM((4, 128, 128), f32),
    pltpu.VMEM((2, 32, 128, 128), f32),
    pltpu.VMEM((2, N_COARSE, 128, 128), f32),
    pltpu.VMEM((NG, L_SEQ + 8, 128), f32),
    pltpu.VMEM((NG, L_SEQ, 128), f32),
    pltpu.VMEM((64, JP // 2, 128), i32),
    pltpu.VMEM((64, 16, 256), i32),
    pltpu.VMEM((64, 128 * (3 if PASSES2 == 3 else 1)), i32),
    pltpu.VMEM((64, 128 * (3 if PASSES2 == 3 else 1)), i32),
    pltpu.VMEM((NG, 64 * JP, 128), f32),
    pltpu.VMEM((NG, 64 * JP, 128), f32),
    pltpu.VMEM((NG, 33 * 128, 128), f32),
    pltpu.VMEM((NG, 64 * 32, 128), f32),
]


def _kernel(x_ref, wqkv_ref, wo_ref, u_ref, are, aim, bre, bim, cre, cim, ldt_ref, dsk_ref, out_ref,
            wqT, wvT, k3, qT3, vT3, oT, bias, *ssm_scratch):
    if PH != 'B':
        _attention_part(x_ref, wqkv_ref, wo_ref, out_ref, wqT, wvT, k3, qT3, vT3, oT, bias)
    else:
        out_ref[:, pl.ds(0, D_MODEL)] = jnp.zeros((S_LEN, D_MODEL), bf16)
    if PH != 'A':
        _ssm_part(u_ref, (are, aim, bre, bim, cre, cim), ldt_ref, dsk_ref, out_ref, *ssm_scratch)
    else:
        out_ref[:, pl.ds(D_MODEL, D_MODEL)] = jnp.zeros((S_LEN, D_MODEL), bf16)


@jax.jit
def pallas_concat_heads__sliding_block__ssm_conv_s4__prompt_kernel(
    A_x: jax.Array,
    A_wqkv: jax.Array,
    A_wo: jax.Array,
    B_u: jax.Array,
    B_A_re: jax.Array,
    B_A_im: jax.Array,
    B_B_re: jax.Array,
    B_B_im: jax.Array,
    B_C_re: jax.Array,
    B_C_im: jax.Array,
    B_log_dt: jax.Array,
    B_Dskip: jax.Array,
):
    x = A_x.reshape(S_LEN, D_MODEL)
    scratch = [
        pltpu.VMEM((D_MODEL, D_MODEL), bf16),
        pltpu.VMEM((D_MODEL, D_MODEL), bf16),
        pltpu.VMEM((NG, S_LEN, 128), bf16),
        pltpu.VMEM((NQB, D_MODEL, QB), bf16),
        pltpu.VMEM((NQB, D_MODEL, QB), bf16),
        pltpu.VMEM((D_MODEL, QB), bf16),
        pltpu.VMEM((2, QB, QB), f32),
    ]
    out = pl.pallas_call(
        _kernel,
        out_shape=jax.ShapeDtypeStruct((S_LEN, 2 * D_MODEL), bf16),
        scratch_shapes=scratch + _SSM_SCRATCH,
        compiler_params=pltpu.CompilerParams(vmem_limit_bytes=110 * 1024 * 1024),
    )(x, A_wqkv, A_wo, B_u.reshape(L_SEQ, D_MODEL), B_A_re, B_A_im, B_B_re, B_B_im, B_C_re, B_C_im,
      B_log_dt.reshape(NG, 1, 128), B_Dskip.reshape(NG, 1, 128))
    return out.reshape(1, S_LEN, 2 * D_MODEL)
```

```python
import functools
import math

import numpy as np
import jax
import jax.numpy as jnp
from jax import lax
import jax.experimental.pallas as pl
import jax.experimental.pallas.tpu as pltpu

f32 = jnp.float32
bf16 = jnp.bfloat16
i32 = jnp.int32

S_LEN = 2048
D_MODEL = 512
N_HEADS = 32
D_HEAD = 16
WINDOW = 256
QB = 128
NQB = S_LEN // QB
NG = 4
NEG = -1e9
PH = 'all'
SP = 'end'


def _dot(a, b):
    return jnp.dot(a, b, preferred_element_type=f32)


def _dot_nt(a, b):
    return lax.dot_general(a, b, (((1,), (1,)), ((), ())), preferred_element_type=f32)


def _dot_tn(a, b):
    return lax.dot_general(a, b, (((0,), (0,)), ((), ())), preferred_element_type=f32)


def _attention_part(x_ref, wqkv_ref, wo_ref, out_ref, wqT, wvT, k3, qT3, vT3, oT, bias, sS, mS, pS, lS, pmask):
    for (col0, dst) in ((0, wqT), (2 * D_MODEL, wvT)):
        for r in range(4):
            for c in range(4):
                blk = wqkv_ref[pl.ds(128 * r, 128), pl.ds(col0 + 128 * c, 128)].astype(f32)
                dst[pl.ds(128 * c, 128), pl.ds(128 * r, 128)] = blk.T.astype(bf16)

    rr = lax.broadcasted_iota(i32, (QB, QB), 0)
    cc = lax.broadcasted_iota(i32, (QB, QB), 1)
    bias[...] = jnp.where(rr <= cc, 0.0, NEG).astype(f32)
    r2 = lax.broadcasted_iota(i32, (QB // 2, QB), 0) * 2
    c2 = lax.broadcasted_iota(i32, (QB // 2, QB), 1)
    mt = jnp.where(r2 > c2, 0xFFFF, 0) | jnp.where(r2 + 1 > c2, -65536, 0)
    pmask[0] = mt
    pmask[1] = ~mt

    wk = wqkv_ref[:, pl.ds(D_MODEL, D_MODEL)]

    def proj_body(i, c):
        r0 = pl.multiple_of(i * QB, QB)
        xb = x_ref[pl.ds(r0, QB), :]
        kb = _dot(xb, wk).astype(bf16)
        for g in range(NG):
            k3[g, pl.ds(r0, QB), :] = kb[:, 128 * g:128 * (g + 1)]
        qT3[i] = (_dot_nt(wqT[...], xb) * (D_HEAD ** -0.5 * math.log2(math.e))).astype(bf16)
        vT3[i] = _dot_nt(wvT[...], xb).astype(bf16)
        return c

    lax.fori_loop(0, NQB, proj_body, 0)
    k3w, qT3w, vT3w, pSw = (r.bitcast(i32) for r in (k3, qT3, vT3, pS))

    def attend(i, nblk):
        R = QB * min(nblk, 2)

        def phase1(g, c):
            kr0 = pl.multiple_of((i - nblk + 1) * (QB // 2), QB // 2)
            for hh in range(8):
                h = 8 * g + hh
                qh = qT3w[i, pl.ds(64 * g + 8 * hh, 8), :]
                pieces = []
                if hh > 0:
                    pieces.append(jnp.zeros((8 * hh, QB), i32))
                pieces.append(qh)
                if hh < 7:
                    pieces.append(jnp.zeros((56 - 8 * hh, QB), i32))
                qsel = _from_packed(jnp.concatenate(pieces, axis=0))
                sb = [_dot(_from_packed(k3w[g, pl.ds(kr0 + 64 * j, 64), :]), qsel) for j in range(nblk)]
                if nblk == 3:
                    blocks = [sb[1], jnp.where(rr > cc, sb[0], sb[2])]
                elif nblk == 2:
                    blocks = [sb[0], sb[1] + bias[...]]
                else:
                    blocks = [sb[0] + bias[...]]
                m = blocks[0].max(axis=0, keepdims=True)
                for b in blocks[1:]:
                    m = jnp.maximum(m, b.max(axis=0, keepdims=True))
                l = None
                for j, b in enumerate(blocks):
                    p = jnp.exp2(b - m)
                    ps = p.sum(axis=0, keepdims=True)
                    l = ps if l is None else l + ps
                    pS[h, pl.ds(QB * j, QB), :] = p.astype(bf16)
                lS[h] = l
            return c

        lax.fori_loop(0, NG, phase1, 0)

        def phase3(g, c):
            for hh in range(8):
                h = 8 * g + hh
                dr = pl.ds(64 * g + 8 * hh, 8)
                if nblk == 3:
                    pg = pSw[h, pl.ds(64, 64), :]
                    rhs = jnp.concatenate([pg & pmask[0], pSw[h, pl.ds(0, 64), :], pg & pmask[1]], axis=0)
                else:
                    rhs = pSw[h, pl.ds(0, R // 2), :]
                lhs = jnp.concatenate([vT3w[i - nblk + 1 + j, dr, :] for j in range(nblk)], axis=1)
                o = _dot(_from_packed(lhs), _from_packed(rhs))
                oT[pl.ds(128 * g + 16 * hh, 16), :] = (o / lS[h]).astype(bf16)
            return c

        lax.fori_loop(0, NG, phase3, 0)
        r0 = pl.multiple_of(i * QB, QB)
        out_ref[pl.ds(r0, QB), pl.ds(0, D_MODEL)] = _dot_tn(oT[...], wo_ref[...]).astype(bf16)

    attend(0, 1)
    attend(1, 2)

    def attn_body(i, c):
        attend(i, 3)
        return c

    lax.fori_loop(2, NQB, attn_body, 0)


L_SEQ = 2048
M_FFT = 4096
NJ = 66
JP = 80
PASSES2 = 3

_P1 = 1.5703125
_P2 = 4.837512969970703125e-4
_P3 = 7.54978995489188216e-8


def _sincos_poly(r):
    r2 = r * r
    s = r + r * r2 * (-1.6666654611e-1 + r2 * (8.3321608736e-3 + r2 * (-1.9515295891e-4)))
    c = 1.0 - 0.5 * r2 + r2 * r2 * (4.166664568298827e-2 + r2 * (-1.388731625493765e-3 + r2 * 2.443315711809948e-5))
    return s, c


def _quadrant_fix(q, s, c):
    swap = (q & 1) == 1
    sn = jnp.where(swap, c, s)
    cs = jnp.where(swap, s, c)
    sn = jnp.where((q & 2) == 2, -sn, sn)
    cs = jnp.where(((q + 1) & 2) == 2, -cs, cs)
    return cs, sn


def _cis(theta):
    qf = jnp.floor(theta * (2.0 / math.pi) + 0.5)
    r = theta - qf * _P1
    r = r - qf * _P2
    r = r - qf * _P3
    s, c = _sincos_poly(r)
    return _quadrant_fix(qf.astype(i32), s, c)


def _trig_int(m):
    q = (m + 512) >> 10
    r = (m - (q << 10)).astype(f32) * (2.0 * math.pi / M_FFT)
    s, c = _sincos_poly(r)
    return _quadrant_fix(q, s, c)


def _hi(x):
    return lax.bitcast_convert_type(lax.bitcast_convert_type(x, i32) & jnp.int32(-65536), f32)


def _to_packed(x_f32):
    return pltpu.bitcast(x_f32.astype(bf16), i32)


def _from_packed(x_i32):
    return pltpu.bitcast(x_i32, bf16)


def _plan_powers():
    direct = (1, 8, 64, 512)
    have, ops = set(), []

    def ensure(e):
        if e in have:
            return
        if e in direct:
            ops.append(("direct", e))
        elif e & (e - 1) == 0:
            ensure(e // 2)
            ops.append(("sq", e, e // 2))
        else:
            hb = 1 << (e.bit_length() - 1)
            ensure(hb)
            ensure(e - hb)
            ops.append(("mul", e, hb, e - hb))
        have.add(e)

    for s in (1, 2, 4, 8):
        for b in range(1, 8):
            ensure(s * b)
        for b in range(1, 8):
            ensure(8 * s * b)
    for e in (64, 128, 192, 256, 512, 1024, 2048):
        ensure(e)
    return ops


_POWER_PLAN = _plan_powers()
N_COARSE = 81
N_BLOCKS = 20
NA = 4


def _build_dft_tables(t1, t3, f2, f2i):
    ncol = 128 * (3 if PASSES2 == 3 else 1)
    row = lax.broadcasted_iota(i32, (128, ncol), 0)
    col = lax.broadcasted_iota(i32, (128, ncol), 1)
    p = col >> 7
    ci = col & 127
    po, k2 = row >> 6, row & 63
    pi_, n2 = ci >> 6, ci & 63
    c, s = _trig_int(((k2 * n2) & 63) << 6)
    for dst, sgn in ((f2, 1.0), (f2i, -1.0)):
        val = jnp.where(po == pi_, c, jnp.where(po == 0, sgn * s, -sgn * s))
        hi = val.astype(bf16).astype(f32)
        dst[...] = _to_packed(jnp.where(p == 1, val - hi, hi))

    def body(n2, carry):
        row = lax.broadcasted_iota(i32, (JP, 128), 0)
        col = lax.broadcasted_iota(i32, (JP, 128), 1)
        p = col >> 5
        n1 = col & 31
        k1 = row >> 1
        t = (n1 << 6) + n2
        c, s = _trig_int((k1 * t) & (M_FFT - 1))
        val = jnp.where((row & 1) == 0, c, -s)
        val = jnp.where((row < NJ) & (p < 3), val, 0.0)
        hi = val.astype(bf16).astype(f32)
        t1[n2] = _to_packed(jnp.where(p == 1, val - hi, hi))
        row = lax.broadcasted_iota(i32, (32, 256), 0)
        col = lax.broadcasted_iota(i32, (32, 256), 1)
        p = (col >= JP).astype(i32) + (col >= 2 * JP).astype(i32) + (col >= 3 * JP).astype(i32)
        j = col - JP * p
        k1 = j >> 1
        t = (row << 6) + n2
        c, s = _trig_int((k1 * t) & (M_FFT - 1))
        val = jnp.where((j & 1) == 0, c, -s)
        w = jnp.where((k1 == 0) | (k1 == 32), 1.0 / M_FFT, 2.0 / M_FFT)
        val = jnp.where((j < NJ) & (p < 3), val * w, 0.0)
        hi = val.astype(bf16).astype(f32)
        t3[n2] = _to_packed(jnp.where(p == 1, val - hi, hi))
        return carry

    lax.fori_loop(0, 64, body, 0)


def _cmul(a, b):
    return a[0] * b[0] - a[1] * b[1], a[0] * b[1] + a[1] * b[0]


def _kgen_group(g, prm_refs, ldt_ref, lam, tabF, tabC, kall):
    are, aim, bre, bim, cre, cim = prm_refs
    r0 = pl.multiple_of(g * 128, 128)
    dt = jnp.exp(ldt_ref[g].astype(f32)).astype(bf16).astype(f32)

    def tr(ref):
        return ref[pl.ds(r0, 128), :].astype(f32).T

    dbr = tr(bre) * dt
    dbi = tr(bim) * dt
    cr_, ci_ = tr(cre), tr(cim)
    lam[0] = tr(are) * dt
    lam[1] = tr(aim) * dt
    lam[2] = cr_ * dbr - ci_ * dbi
    lam[3] = cr_ * dbi + ci_ * dbr

    CH = 16

    def tab_body(ch, carry):
        rows = pl.ds(pl.multiple_of(ch * CH, CH), CH)
        lr, li = lam[0, rows, :], lam[1, rows, :]
        cc = (lam[2, rows, :], lam[3, rows, :])
        W = {}
        for op in _POWER_PLAN:
            if op[0] == "direct":
                e = float(op[1])
                mag = jnp.exp(lr * e)
                c, s = _cis(li * e)
                W[op[1]] = (mag * c, mag * s)
            elif op[0] == "sq":
                a, b = W[op[2]]
                W[op[1]] = (a * a - b * b, (a + a) * b)
            else:
                W[op[1]] = _cmul(W[op[2]], W[op[3]])
        for si, s in enumerate((1, 2, 4, 8)):
            for b in range(1, 8):
                tabF[0, 8 * si + b, rows, :] = W[s * b][0]
                tabF[1, 8 * si + b, rows, :] = W[s * b][1]

        def put(idx, v):
            tabC[0, idx, rows, :] = v[0]
            tabC[1, idx, rows, :] = v[1]

        base = cc
        for p in range(4):
            if p > 0:
                base = _cmul(cc, W[64 * p])
            put(8 * p, base)
            for i in range(1, 8):
                put(8 * p + i, _cmul(base, W[8 * i]))
        for si, s in ((1, 2), (2, 4), (3, 8)):
            base = _cmul(cc, W[128 * s])
            for p in range(2):
                if p == 1:
                    base = _cmul(base, W[64 * s])
                o = 32 + 16 * (si - 1) + 8 * p
                put(o, base)
                for i in range(1, 8):
                    put(o + i, _cmul(base, W[8 * s * i]))
        put(80, _cmul(cc, W[2048]))
        return carry

    lax.fori_loop(0, 128 // CH, tab_body, 0)

    def blk_body(kk, carry):
        nb0 = 32 // NA
        nbs = 16 // NA
        si = jnp.where(kk < nb0, 0, 1 + (kk - nb0) // nbs)
        a0 = jnp.where(kk < nb0, NA * kk, 16 + NA * ((kk - nb0) % nbs))
        step = jnp.left_shift(1, si)
        fbase = 8 * si
        acc = [[None] * 8 for _ in range(NA)]
        for nb in range(16):
            rows = pl.ds(8 * nb, 8)
            cr = [tabC[0, NA * kk + a, rows, :] for a in range(NA)]
            ci = [tabC[1, NA * kk + a, rows, :] for a in range(NA)]
            for b in range(8):
                if b > 0:
                    fr = tabF[0, fbase + b, rows, :]
                    fi = tabF[1, fbase + b, rows, :]
                for a in range(NA):
                    term = cr[a] if b == 0 else cr[a] * fr - ci[a] * fi
                    acc[a][b] = term if nb == 0 else acc[a][b] + term
        for a in range(NA):
            for b in range(8):
                row = step * (8 * (a0 + a) + b)
                kall[g, pl.ds(row, 1), :] = jnp.sum(acc[a][b], axis=0, keepdims=True)
        return carry

    lax.fori_loop(0, 80 // NA, blk_body, 0)
    kall[g, pl.ds(L_SEQ, 1), :] = jnp.sum(tabC[0, 80], axis=0, keepdims=True)


def _split_rhs(x, extra_zero_rows=0):
    xh = _hi(x)
    pieces = [xh, xh, x - xh]
    if extra_zero_rows:
        pieces.append(jnp.zeros((extra_zero_rows, x.shape[1]), f32))
    return jnp.concatenate(pieces, axis=0).astype(bf16)


def _round_off(n2, s):
    q = n2 // s
    rem = n2 - q * s
    up = (rem * 2 > s) | ((rem * 2 == s) & ((q & 1) == 1))
    return (q + up.astype(i32)) * s


def _ssm_part(u_ref, prm_refs, ldt_ref, dsk_ref, out_ref,
              lam, tabF, tabC, kall, uf, t1, t3, f2, f2i, bsu, bsk, zs, yp, ys):
    for g in range(NG):
        uf[g] = u_ref[:, pl.ds(128 * g, 128)].astype(f32)

    if SP == 'tables':
        out_ref[:, pl.ds(D_MODEL, D_MODEL)] = jnp.zeros((S_LEN, D_MODEL), bf16)
        return

    def kg(g, c):
        _kgen_group(g, prm_refs, ldt_ref, lam, tabF, tabC, kall)
        return c

    lax.fori_loop(0, NG, kg, 0)

    if SP == 'kgen':
        out_ref[:, pl.ds(D_MODEL, D_MODEL)] = jnp.zeros((S_LEN, D_MODEL), bf16)
        return
    def st1_body(n2, carry):
        lhs = _from_packed(t1[n2])
        o = pl.multiple_of(n2 * JP, 16)
        xu = jnp.concatenate([uf[g, pl.ds(n2, 32, stride=64), :] for g in range(NG)], axis=1)
        bu = _dot(lhs, _split_rhs(xu, 32))
        o2, o4, o8 = 256 + _round_off(n2, 2), 512 + _round_off(n2, 4), 1024 + _round_off(n2, 8)
        xk = jnp.concatenate([jnp.concatenate([
            kall[g, pl.ds(n2, 4, stride=64), :],
            kall[g, pl.ds(o2, 4, stride=64), :],
            kall[g, pl.ds(o4, 8, stride=64), :],
            kall[g, pl.ds(o8, 16, stride=64), :]], axis=0) for g in range(NG)], axis=1)
        bk = _dot(lhs, _split_rhs(xk, 32))
        for g in range(NG):
            bsu[g, pl.ds(o, JP), :] = bu[:, 128 * g:128 * (g + 1)]
            bsk[g, pl.ds(o, JP), :] = bk[:, 128 * g:128 * (g + 1)]
        return carry

    lax.fori_loop(0, 64, st1_body, 0, unroll=4)

    if SP == 'st1':
        out_ref[:, pl.ds(D_MODEL, D_MODEL)] = jnp.zeros((S_LEN, D_MODEL), bf16)
        return
    def prep(x):
        if PASSES2 == 3:
            return _split_rhs(x)
        return x.astype(bf16)

    def gather128(bs, k1):
        return jnp.concatenate([
            jnp.concatenate([bs[g, pl.ds(2 * k1, 64, stride=JP), :],
                             bs[g, pl.ds(2 * k1 + 1, 64, stride=JP), :]], axis=0)
            for g in range(NG)], axis=1)

    def k1f_body(k1, carry):
        lf = _from_packed(f2[...])
        xu = _dot(lf, prep(gather128(bsu, k1)))
        xk = _dot(lf, prep(gather128(bsk, k1)))
        ur, ui, kr, ki = xu[:64], xu[64:], xk[:64], xk[64:]
        ys[pl.ds(pl.multiple_of(k1 * 128, 128), 128), :] = jnp.concatenate(
            [ur * kr - ui * ki, ur * ki + ui * kr], axis=0)
        return carry

    lax.fori_loop(0, 33, k1f_body, 0)

    def k1i_body(k1, carry):
        li = _from_packed(f2i[...])
        r = pl.ds(pl.multiple_of(k1 * 128, 128), 128)
        z = _dot(li, prep(ys[r, :]))
        for g in range(NG):
            zs[g, r, :] = z[:, 128 * g:128 * (g + 1)]
        return carry

    lax.fori_loop(0, 33, k1i_body, 0)

    if SP == 'k1':
        out_ref[:, pl.ds(D_MODEL, D_MODEL)] = jnp.zeros((S_LEN, D_MODEL), bf16)
        return
    def st3_body(n2, carry):
        lhs = _from_packed(t3[n2])
        z = jnp.concatenate([zs[g, pl.ds(n2, NJ, stride=64), :] for g in range(NG)], axis=1)
        z = jnp.concatenate([z, jnp.zeros((JP - NJ, 128 * NG), f32)], axis=0)
        y = _dot(lhs, _split_rhs(z, 16))
        for g in range(NG):
            yp[g, pl.ds(pl.multiple_of(n2 * 32, 32), 32), :] = y[:, 128 * g:128 * (g + 1)]
        return carry

    lax.fori_loop(0, 64, st3_body, 0, unroll=4)

    if SP == 'st3':
        out_ref[:, pl.ds(D_MODEL, D_MODEL)] = jnp.zeros((S_LEN, D_MODEL), bf16)
        return
    dsk = [dsk_ref[g].astype(f32) for g in range(NG)]

    def ep_body(n1, carry):
        for q in range(4):
            r0 = pl.multiple_of(n1 * 64 + 16 * q, 16)
            for g in range(NG):
                y = jnp.concatenate([yp[g, pl.ds(32 * (16 * q) + n1, 8, stride=32), :],
                                     yp[g, pl.ds(32 * (16 * q + 8) + n1, 8, stride=32), :]], axis=0)
                yb = y.astype(bf16).astype(f32)
                ud = (uf[g, pl.ds(r0, 16), :] * dsk[g]).astype(bf16).astype(f32)
                out_ref[pl.ds(r0, 16), pl.ds(D_MODEL + 128 * g, 128)] = (yb + ud).astype(bf16)
        return carry

    lax.fori_loop(0, 32, ep_body, 0, unroll=2)


_SSM_SCRATCH = [
    pltpu.VMEM((4, 128, 128), f32),
    pltpu.VMEM((2, 32, 128, 128), f32),
    pltpu.VMEM((2, N_COARSE, 128, 128), f32),
    pltpu.VMEM((NG, L_SEQ + 8, 128), f32),
    pltpu.VMEM((NG, L_SEQ, 128), f32),
    pltpu.VMEM((64, JP // 2, 128), i32),
    pltpu.VMEM((64, 16, 256), i32),
    pltpu.VMEM((64, 128 * (3 if PASSES2 == 3 else 1)), i32),
    pltpu.VMEM((64, 128 * (3 if PASSES2 == 3 else 1)), i32),
    pltpu.VMEM((NG, 64 * JP, 128), f32),
    pltpu.VMEM((NG, 64 * JP, 128), f32),
    pltpu.VMEM((NG, 33 * 128, 128), f32),
    pltpu.VMEM((NG, 64 * 32, 128), f32),
    pltpu.VMEM((33 * 128, 512), f32),
]


def _kernel(x_hbm, wqkv_hbm, wo_hbm, u_hbm, are_h, aim_h, bre_h, bim_h, cre_h, cim_h, ldt_ref, dsk_ref, out_hbm,
            xv, wv, wov, uv, pv, outv, sems,
            wqT, wvT, k3, qT3, vT3, oT, bias, sS, mS, pS, lS, pmask, *ssm_scratch):
    in_copies = [pltpu.make_async_copy(src, dst, sems.at[k]) for k, (src, dst) in enumerate((
        (x_hbm, xv), (wqkv_hbm, wv), (wo_hbm, wov), (u_hbm, uv),
        (are_h, pv.at[0]), (aim_h, pv.at[1]), (bre_h, pv.at[2]), (bim_h, pv.at[3]),
        (cre_h, pv.at[4]), (cim_h, pv.at[5])))]
    for cp in in_copies:
        cp.start()
    (lam, tabF, tabC, kall, uf, t1, t3, f2, f2i, bsu, bsk, zs, yp, ys) = ssm_scratch
    _build_dft_tables(t1, t3, f2, f2i)
    for cp in in_copies[:3]:
        cp.wait()
    _attention_part(xv, wv, wov, outv, wqT, wvT, k3, qT3, vT3, oT, bias, sS, mS, pS, lS, pmask)
    out_a = pltpu.make_async_copy(outv.at[:, pl.ds(0, D_MODEL)], out_hbm.at[:, pl.ds(0, D_MODEL)], sems.at[10])
    out_a.start()
    for cp in in_copies[3:]:
        cp.wait()
    _ssm_part(uv, tuple(pv.at[k] for k in range(6)), ldt_ref, dsk_ref, outv, *ssm_scratch)
    out_b = pltpu.make_async_copy(outv.at[:, pl.ds(D_MODEL, D_MODEL)], out_hbm.at[:, pl.ds(D_MODEL, D_MODEL)], sems.at[11])
    out_b.start()
    out_a.wait()
    out_b.wait()


@jax.jit
def pallas_concat_heads__sliding_block__ssm_conv_s4__prompt_kernel(
    A_x: jax.Array,
    A_wqkv: jax.Array,
    A_wo: jax.Array,
    B_u: jax.Array,
    B_A_re: jax.Array,
    B_A_im: jax.Array,
    B_B_re: jax.Array,
    B_B_im: jax.Array,
    B_C_re: jax.Array,
    B_C_im: jax.Array,
    B_log_dt: jax.Array,
    B_Dskip: jax.Array,
):
    x = A_x.reshape(S_LEN, D_MODEL)
    io_scratch = [
        pltpu.VMEM((S_LEN, D_MODEL), bf16),
        pltpu.VMEM((D_MODEL, 3 * D_MODEL), bf16),
        pltpu.VMEM((D_MODEL, D_MODEL), bf16),
        pltpu.VMEM((L_SEQ, D_MODEL), bf16),
        pltpu.VMEM((6, D_MODEL, 128), bf16),
        pltpu.VMEM((S_LEN, 2 * D_MODEL), bf16),
        pltpu.SemaphoreType.DMA((12,)),
    ]
    scratch = [
        pltpu.VMEM((D_MODEL, D_MODEL), bf16),
        pltpu.VMEM((D_MODEL, D_MODEL), bf16),
        pltpu.VMEM((NG, S_LEN, 128), bf16),
        pltpu.VMEM((NQB, D_MODEL, QB), bf16),
        pltpu.VMEM((NQB, D_MODEL, QB), bf16),
        pltpu.VMEM((D_MODEL, QB), bf16),
        pltpu.VMEM((QB, QB), f32),
        pltpu.VMEM((N_HEADS, 2 * QB, QB), f32),
        pltpu.VMEM((N_HEADS, 1, QB), f32),
        pltpu.VMEM((N_HEADS, 2 * QB, QB), bf16),
        pltpu.VMEM((N_HEADS, 1, QB), f32),
        pltpu.VMEM((2, QB // 2, QB), i32),
    ]
    out = pl.pallas_call(
        _kernel,
        out_shape=jax.ShapeDtypeStruct((S_LEN, 2 * D_MODEL), bf16),
        in_specs=[pl.BlockSpec(memory_space=pl.ANY)] * 10 + [pl.BlockSpec(memory_space=pltpu.VMEM)] * 2,
        out_specs=pl.BlockSpec(memory_space=pl.ANY),
        scratch_shapes=io_scratch + scratch + _SSM_SCRATCH,
        compiler_params=pltpu.CompilerParams(vmem_limit_bytes=110 * 1024 * 1024),
    )(x, A_wqkv, A_wo, B_u.reshape(L_SEQ, D_MODEL), B_A_re, B_A_im, B_B_re, B_B_im, B_C_re, B_C_im,
      B_log_dt.reshape(NG, 1, 128), B_Dskip.reshape(NG, 1, 128))
    return out.reshape(1, S_LEN, 2 * D_MODEL)
```

```python
import functools
import math

import numpy as np
import jax
import jax.numpy as jnp
from jax import lax
import jax.experimental.pallas as pl
import jax.experimental.pallas.tpu as pltpu

f32 = jnp.float32
bf16 = jnp.bfloat16
i32 = jnp.int32

S_LEN = 2048
D_MODEL = 512
N_HEADS = 32
D_HEAD = 16
WINDOW = 256
QB = 128
NQB = S_LEN // QB
NG = 4
NEG = -1e9
PH = 'all'
SP = 'end'


def _dot(a, b):
    return jnp.dot(a, b, preferred_element_type=f32)


def _dot_nt(a, b):
    return lax.dot_general(a, b, (((1,), (1,)), ((), ())), preferred_element_type=f32)


def _dot_tn(a, b):
    return lax.dot_general(a, b, (((0,), (0,)), ((), ())), preferred_element_type=f32)


def _attention_part(x_ref, wqkv_ref, wo_ref, out_ref, wqT, wvT, k3, qT3, vT3, oT, bias, sS, mS, pS, lS, pmask, host=None,
                    before_host=None):
    for (col0, dst) in ((0, wqT), (2 * D_MODEL, wvT)):
        for r in range(4):
            for c in range(4):
                blk = wqkv_ref[pl.ds(128 * r, 128), pl.ds(col0 + 128 * c, 128)].astype(f32)
                dst[pl.ds(128 * c, 128), pl.ds(128 * r, 128)] = blk.T.astype(bf16)

    rr = lax.broadcasted_iota(i32, (QB, QB), 0)
    cc = lax.broadcasted_iota(i32, (QB, QB), 1)
    bias[...] = jnp.where(rr <= cc, 0.0, NEG).astype(f32)
    r2 = lax.broadcasted_iota(i32, (QB // 2, QB), 0) * 2
    c2 = lax.broadcasted_iota(i32, (QB // 2, QB), 1)
    mt = jnp.where(r2 > c2, 0xFFFF, 0) | jnp.where(r2 + 1 > c2, -65536, 0)
    pmask[0] = mt
    pmask[1] = ~mt

    wk = wqkv_ref[:, pl.ds(D_MODEL, D_MODEL)]

    def proj_body(i, c):
        r0 = pl.multiple_of(i * QB, QB)
        xb = x_ref[pl.ds(r0, QB), :]
        kb = _dot(xb, wk).astype(bf16)
        for g in range(NG):
            k3[g, pl.ds(r0, QB), :] = kb[:, 128 * g:128 * (g + 1)]
        qT3[i] = (_dot_nt(wqT[...], xb) * (D_HEAD ** -0.5 * math.log2(math.e))).astype(bf16)
        vT3[i] = _dot_nt(wvT[...], xb).astype(bf16)
        return c

    lax.fori_loop(0, NQB, proj_body, 0)
    k3w, qT3w, vT3w, pSw = (r.bitcast(i32) for r in (k3, qT3, vT3, pS))

    def attend(i, nblk):
        R = QB * min(nblk, 2)

        def phase1(g, c):
            hosting = host is not None and nblk == 3
            if hosting:
                micro = host((i - 2) * NG + g)
            kr0 = pl.multiple_of((i - nblk + 1) * (QB // 2), QB // 2)
            for hh in range(8):
                h = 8 * g + hh
                qh = qT3w[i, pl.ds(64 * g + 8 * hh, 8), :]
                pieces = []
                if hh > 0:
                    pieces.append(jnp.zeros((8 * hh, QB), i32))
                pieces.append(qh)
                if hh < 7:
                    pieces.append(jnp.zeros((56 - 8 * hh, QB), i32))
                qsel = _from_packed(jnp.concatenate(pieces, axis=0))
                sb = [_dot(_from_packed(k3w[g, pl.ds(kr0 + 64 * j, 64), :]), qsel) for j in range(nblk)]
                if nblk == 3:
                    blocks = [sb[1], jnp.where(rr > cc, sb[0], sb[2])]
                elif nblk == 2:
                    blocks = [sb[0], sb[1] + bias[...]]
                else:
                    blocks = [sb[0] + bias[...]]
                if hosting:
                    for k in range(MICRO_PER_HEAD):
                        micro(jnp.minimum(jnp.abs(blocks[k % 2][32 * (k // 2):32 * (k // 2) + 8, :]), 0.0))
                m = blocks[0].max(axis=0, keepdims=True)
                for b in blocks[1:]:
                    m = jnp.maximum(m, b.max(axis=0, keepdims=True))
                l = None
                for j, b in enumerate(blocks):
                    p = jnp.exp2(b - m)
                    ps = p.sum(axis=0, keepdims=True)
                    l = ps if l is None else l + ps
                    pS[h, pl.ds(QB * j, QB), :] = p.astype(bf16)
                lS[h] = l
            return c

        lax.fori_loop(0, NG, phase1, 0)

        def phase3(g, c):
            for hh in range(8):
                h = 8 * g + hh
                dr = pl.ds(64 * g + 8 * hh, 8)
                if nblk == 3:
                    pg = pSw[h, pl.ds(64, 64), :]
                    rhs = jnp.concatenate([pg & pmask[0], pSw[h, pl.ds(0, 64), :], pg & pmask[1]], axis=0)
                else:
                    rhs = pSw[h, pl.ds(0, R // 2), :]
                lhs = jnp.concatenate([vT3w[i - nblk + 1 + j, dr, :] for j in range(nblk)], axis=1)
                o = _dot(_from_packed(lhs), _from_packed(rhs))
                oT[pl.ds(128 * g + 16 * hh, 16), :] = (o / lS[h]).astype(bf16)
            return c

        lax.fori_loop(0, NG, phase3, 0)
        r0 = pl.multiple_of(i * QB, QB)
        out_ref[pl.ds(r0, QB), pl.ds(0, D_MODEL)] = _dot_tn(oT[...], wo_ref[...]).astype(bf16)

    attend(0, 1)
    attend(1, 2)
    if before_host is not None:
        before_host()

    def attn_body(i, c):
        attend(i, 3)
        return c

    lax.fori_loop(2, NQB, attn_body, 0)


L_SEQ = 2048
M_FFT = 4096
NJ = 66
JP = 80
JZ = 72
PASSES2 = 3

_P1 = 1.5703125
_P2 = 4.837512969970703125e-4
_P3 = 7.54978995489188216e-8


def _sincos_poly(r):
    r2 = r * r
    s = r + r * r2 * (-1.6666654611e-1 + r2 * (8.3321608736e-3 + r2 * (-1.9515295891e-4)))
    c = 1.0 - 0.5 * r2 + r2 * r2 * (4.166664568298827e-2 + r2 * (-1.388731625493765e-3 + r2 * 2.443315711809948e-5))
    return s, c


def _quadrant_fix(q, s, c):
    swap = (q & 1) == 1
    sn = jnp.where(swap, c, s)
    cs = jnp.where(swap, s, c)
    sn = jnp.where((q & 2) == 2, -sn, sn)
    cs = jnp.where(((q + 1) & 2) == 2, -cs, cs)
    return cs, sn


def _cis(theta):
    qf = jnp.floor(theta * (2.0 / math.pi) + 0.5)
    r = theta - qf * _P1
    r = r - qf * _P2
    r = r - qf * _P3
    s, c = _sincos_poly(r)
    return _quadrant_fix(qf.astype(i32), s, c)


def _trig_int(m):
    q = (m + 512) >> 10
    r = (m - (q << 10)).astype(f32) * (2.0 * math.pi / M_FFT)
    s, c = _sincos_poly(r)
    return _quadrant_fix(q, s, c)


def _hi(x):
    return lax.bitcast_convert_type(lax.bitcast_convert_type(x, i32) & jnp.int32(-65536), f32)


def _to_packed(x_f32):
    return pltpu.bitcast(x_f32.astype(bf16), i32)


def _from_packed(x_i32):
    return pltpu.bitcast(x_i32, bf16)


def _plan_powers():
    direct = (1, 8, 64, 512)
    have, ops = set(), []

    def ensure(e):
        if e in have:
            return
        if e in direct:
            ops.append(("direct", e))
        elif e & (e - 1) == 0:
            ensure(e // 2)
            ops.append(("sq", e, e // 2))
        else:
            hb = 1 << (e.bit_length() - 1)
            ensure(hb)
            ensure(e - hb)
            ops.append(("mul", e, hb, e - hb))
        have.add(e)

    for s in (1, 2, 4, 8):
        for b in range(1, 8):
            ensure(s * b)
        for b in range(1, 8):
            ensure(8 * s * b)
    for e in (64, 128, 192, 256, 512, 1024, 2048):
        ensure(e)
    return ops


_POWER_PLAN = _plan_powers()
N_COARSE = 81
N_BLOCKS = 20
NA = 2
MICRO_PER_HEAD = 4
BLK_PER_BODY = MICRO_PER_HEAD // 2


def _build_dft_tables(t1, t3, f2, f2i, tq1, tq3):
    ncol = 128 * (3 if PASSES2 == 3 else 1)
    row = lax.broadcasted_iota(i32, (128, ncol), 0)
    col = lax.broadcasted_iota(i32, (128, ncol), 1)
    p = col >> 7
    ci = col & 127
    po, k2 = row >> 6, row & 63
    pi_, n2 = ci >> 6, ci & 63
    c, s = _trig_int(((k2 * n2) & 63) << 6)
    for dst, sgn in ((f2, 1.0), (f2i, -1.0)):
        val = jnp.where(po == pi_, c, jnp.where(po == 0, sgn * s, -sgn * s))
        hi = val.astype(bf16).astype(f32)
        dst[...] = _to_packed(jnp.where(p == 1, val - hi, hi))

    r1 = lax.broadcasted_iota(i32, (JP, 128), 0)
    c1 = lax.broadcasted_iota(i32, (JP, 128), 1)
    k1_1 = r1 >> 1
    ca1, sa1 = _trig_int((k1_1 * ((c1 & 31) << 6)) & (M_FFT - 1))
    r3 = lax.broadcasted_iota(i32, (32, 256), 0)
    c3 = lax.broadcasted_iota(i32, (32, 256), 1)
    p3 = (c3 >= JZ).astype(i32) + (c3 >= 2 * JZ).astype(i32) + (c3 >= 3 * JZ).astype(i32)
    j3 = c3 - JZ * p3
    k1_3 = j3 >> 1
    ca3, sa3 = _trig_int((k1_3 * (r3 << 6)) & (M_FFT - 1))
    for b in range(8):
        tq1[0, b], tq1[1, b] = _trig_int(k1_1 * b)
        tq3[0, b], tq3[1, b] = _trig_int(k1_3 * b)

    def body(a, carry):
        pc1, ps1 = _trig_int(k1_1 * (8 * a))
        pc3, ps3 = _trig_int(k1_3 * (8 * a))
        for b in range(8):
            n2 = 8 * a + b
            bc, bs = _cmul((pc1, ps1), (tq1[0, b], tq1[1, b]))
            c, sn = _cmul((ca1, sa1), (bc, bs))
            val = jnp.where((r1 & 1) == 0, c, -sn)
            val = jnp.where((r1 < NJ) & (c1 < 96), val, 0.0)
            hi = val.astype(bf16).astype(f32)
            t1[n2] = _to_packed(jnp.where((c1 >> 5) == 1, val - hi, hi))
            bc, bs = _cmul((pc3, ps3), (tq3[0, b], tq3[1, b]))
            c, sn = _cmul((ca3, sa3), (bc, bs))
            val = jnp.where((j3 & 1) == 0, c, -sn)
            w = jnp.where((k1_3 == 0) | (k1_3 == 32), 1.0 / M_FFT, 2.0 / M_FFT)
            val = jnp.where((j3 < NJ) & (p3 < 3), val * w, 0.0)
            hi = val.astype(bf16).astype(f32)
            t3[n2] = _to_packed(jnp.where(p3 == 1, val - hi, hi))
        return carry

    lax.fori_loop(0, 8, body, 0)


def _cmul(a, b):
    return a[0] * b[0] - a[1] * b[1], a[0] * b[1] + a[1] * b[0]


def _kgen_prep(g, prm_refs, ldt_ref, lam, tabF, tabC, kall):
    are, aim, bre, bim, cre, cim = prm_refs
    r0 = pl.multiple_of(g * 128, 128)
    dt = jnp.exp(ldt_ref[g].astype(f32)).astype(bf16).astype(f32)

    def tr(ref):
        return ref[pl.ds(r0, 128), :].astype(f32).T

    dbr = tr(bre) * dt
    dbi = tr(bim) * dt
    cr_, ci_ = tr(cre), tr(cim)
    lam[0] = tr(are) * dt
    lam[1] = tr(aim) * dt
    lam[2] = cr_ * dbr - ci_ * dbi
    lam[3] = cr_ * dbi + ci_ * dbr

    CH = 16

    def tab_body(ch, carry):
        rows = pl.ds(pl.multiple_of(ch * CH, CH), CH)
        lr, li = lam[0, rows, :], lam[1, rows, :]
        cc = (lam[2, rows, :], lam[3, rows, :])
        W = {}
        for op in _POWER_PLAN:
            if op[0] == "direct":
                e = float(op[1])
                mag = jnp.exp(lr * e)
                c, s = _cis(li * e)
                W[op[1]] = (mag * c, mag * s)
            elif op[0] == "sq":
                a, b = W[op[2]]
                W[op[1]] = (a * a - b * b, (a + a) * b)
            else:
                W[op[1]] = _cmul(W[op[2]], W[op[3]])
        for si, s in enumerate((1, 2, 4, 8)):
            for b in range(1, 8):
                tabF[0, 8 * si + b, rows, :] = W[s * b][0]
                tabF[1, 8 * si + b, rows, :] = W[s * b][1]

        def put(idx, v):
            tabC[0, idx, rows, :] = v[0]
            tabC[1, idx, rows, :] = v[1]

        base = cc
        for p in range(4):
            if p > 0:
                base = _cmul(cc, W[64 * p])
            put(8 * p, base)
            for i in range(1, 8):
                put(8 * p + i, _cmul(base, W[8 * i]))
        for si, s in ((1, 2), (2, 4), (3, 8)):
            base = _cmul(cc, W[128 * s])
            for p in range(2):
                if p == 1:
                    base = _cmul(base, W[64 * s])
                o = 32 + 16 * (si - 1) + 8 * p
                put(o, base)
                for i in range(1, 8):
                    put(o + i, _cmul(base, W[8 * s * i]))
        put(80, _cmul(cc, W[2048]))
        return carry

    lax.fori_loop(0, 128 // CH, tab_body, 0)
    kall[g, pl.ds(L_SEQ, 1), :] = jnp.sum(tabC[0, 80], axis=0, keepdims=True)


NBLK_G = 80 // NA


class _KgenBlock:
    def __init__(self, item, tabF, tabC, kall):
        self.tabF, self.tabC, self.kall = tabF, tabC, kall
        self.g = item // NBLK_G
        kk = item - self.g * NBLK_G
        nb0 = 32 // NA
        nbs = 16 // NA
        si = jnp.where(kk < nb0, 0, 1 + (kk - nb0) // nbs)
        self.a0 = jnp.where(kk < nb0, NA * kk, 16 + NA * ((kk - nb0) % nbs))
        self.step_ = jnp.left_shift(1, si)
        self.fbase = 8 * si
        self.kk = kk
        self.acc = [[None] * 8 for _ in range(NA)]

    def step(self, nb, zdep=None):
        tabF, tabC, acc = self.tabF, self.tabC, self.acc
        rows = pl.ds(8 * nb, 8)
        cr = [tabC[0, NA * self.kk + a, rows, :] for a in range(NA)]
        ci = [tabC[1, NA * self.kk + a, rows, :] for a in range(NA)]
        if zdep is not None:
            cr = [c + zdep for c in cr]
        for b in range(8):
            if b > 0:
                fr = tabF[0, self.fbase + b, rows, :]
                fi = tabF[1, self.fbase + b, rows, :]
            for a in range(NA):
                term = cr[a] if b == 0 else cr[a] * fr - ci[a] * fi
                acc[a][b] = term if nb == 0 else acc[a][b] + term

    def finish(self):
        for a in range(NA):
            for b in range(8):
                row = self.step_ * (8 * (self.a0 + a) + b)
                self.kall[self.g, pl.ds(row, 1), :] = jnp.sum(self.acc[a][b], axis=0, keepdims=True)


def _kgen_maybe_prep(item, prm_refs, ldt_ref, lam, tabF, tabC, kall):
    g = item // NBLK_G

    @pl.when(item - g * NBLK_G == 0)
    def _():
        _kgen_prep(g, prm_refs, ldt_ref, lam, tabF, tabC, kall)


def _kgen_item(item, tabF, tabC, kall):
    blk = _KgenBlock(item, tabF, tabC, kall)
    for nb in range(16):
        blk.step(nb)
    blk.finish()


def _split_rhs(x, extra_zero_rows=0):
    xh = _hi(x)
    pieces = [xh, xh, x - xh]
    if extra_zero_rows:
        pieces.append(jnp.zeros((extra_zero_rows, x.shape[1]), f32))
    return jnp.concatenate(pieces, axis=0).astype(bf16)


def _block_t(v):
    return jnp.swapaxes(v.reshape(8, 8, v.shape[1]), 0, 1).reshape(64, v.shape[1])


def _round_off(n2, s):
    q = n2 // s
    rem = n2 - q * s
    up = (rem * 2 > s) | ((rem * 2 == s) & ((q & 1) == 1))
    return (q + up.astype(i32)) * s


def _out_b_copy(outv, out_hbm, osems, c):
    r = pl.ds(pl.multiple_of(c * 64, 64), 64)
    cols = pl.ds(D_MODEL, D_MODEL)
    return pltpu.make_async_copy(outv.at[r, cols], out_hbm.at[r, cols], osems.at[c])


def _ssm_part(u_ref, prm_refs, ldt_ref, dsk_ref, out_ref, out_hbm, osems,
              lam, tabF, tabC, kall, uf, t1, t3, f2, f2i, bsu, bsk, zt, yp, ys, tq1, tq3):
    for g in range(NG):
        uf[g] = u_ref[:, pl.ds(128 * g, 128)].astype(f32)

    if SP == 'tables':
        out_ref[:, pl.ds(D_MODEL, D_MODEL)] = jnp.zeros((S_LEN, D_MODEL), bf16)
        return

    def kg(item, c):
        _kgen_maybe_prep(item, prm_refs, ldt_ref, lam, tabF, tabC, kall)
        _kgen_item(item, tabF, tabC, kall)
        return c

    lax.fori_loop((NQB - 2) * NG * BLK_PER_BODY, NG * NBLK_G, kg, 0)

    if SP == 'kgen':
        out_ref[:, pl.ds(D_MODEL, D_MODEL)] = jnp.zeros((S_LEN, D_MODEL), bf16)
        return
    def st1_body(o, carry):
        o8 = pl.multiple_of(o * 8, 8)
        tu = []
        for r in range(4):
            v = jnp.concatenate([
                jnp.concatenate([uf[g, pl.ds(64 * (8 * r + n1) + o8, 8), :] for g in range(NG)], axis=1)
                for n1 in range(8)], axis=0)
            tu.append(_block_t(v))
        for name in ("u", "k"):
            res = []
            for n2l in range(8):
                n2 = o8 + n2l
                if name == "u":
                    x = jnp.concatenate([tu[r][8 * n2l:8 * n2l + 8] for r in range(4)], axis=0)
                else:
                    o2, o4, o8_ = 256 + _round_off(n2, 2), 512 + _round_off(n2, 4), 1024 + _round_off(n2, 8)
                    x = jnp.concatenate([jnp.concatenate([
                        kall[g, pl.ds(n2, 4, stride=64), :],
                        kall[g, pl.ds(o2, 4, stride=64), :],
                        kall[g, pl.ds(o4, 8, stride=64), :],
                        kall[g, pl.ds(o8_, 16, stride=64), :]], axis=0) for g in range(NG)], axis=1)
                res.append(_dot(_from_packed(t1[n2]), _split_rhs(x, 32)))
            dst = bsu if name == "u" else bsk
            for q in range(9):
                t = _block_t(jnp.concatenate([res[n2l][8 * q:8 * q + 8] for n2l in range(8)], axis=0))
                for jj in range(8):
                    if 8 * q + jj < NJ:
                        for g in range(NG):
                            dst[g, pl.ds(64 * (8 * q + jj) + o8, 8), :] = t[8 * jj:8 * jj + 8, 128 * g:128 * (g + 1)]
        return carry

    lax.fori_loop(0, 8, st1_body, 0)

    def prep(x):
        if PASSES2 == 3:
            return _split_rhs(x)
        return x.astype(bf16)

    def wide(ref, rows):
        return jnp.concatenate([ref[g, rows, :] for g in range(NG)], axis=1)

    def k1f_body(k1, carry):
        lf = _from_packed(f2[...])
        r = pl.ds(pl.multiple_of(k1 * 128, 128), 128)
        xu = _dot(lf, prep(wide(bsu, r)))
        xk = _dot(lf, prep(wide(bsk, r)))
        ur, ui, kr, ki = xu[:64], xu[64:], xk[:64], xk[64:]
        ys[r, :] = jnp.concatenate([ur * kr - ui * ki, ur * ki + ui * kr], axis=0)
        return carry

    lax.fori_loop(0, 33, k1f_body, 0, unroll=3)

    def put_zt(blocks, q):
        for o in range(8):
            t = _block_t(jnp.concatenate([b[8 * o:8 * o + 8] for b in blocks], axis=0))
            for n2l in range(8):
                for g in range(NG):
                    zt[g, pl.ds((8 * o + n2l) * JZ + 8 * q, 8), :] = t[8 * n2l:8 * n2l + 8, 128 * g:128 * (g + 1)]

    def k1i_body(q, carry):
        li = _from_packed(f2i[...])
        blocks = []
        for a in range(4):
            z = _dot(li, prep(ys[pl.ds(pl.multiple_of((4 * q + a) * 128, 128), 128), :]))
            blocks += [z[:64], z[64:]]
        put_zt(blocks, q)
        return carry

    lax.fori_loop(0, 8, k1i_body, 0)
    z = _dot(_from_packed(f2i[...]), prep(ys[pl.ds(32 * 128, 128), :]))
    put_zt([z[:64], z[64:]] + [jnp.zeros((64, 128 * NG), f32)] * 6, 8)

    def st3_body(o, carry):
        o8 = pl.multiple_of(o * 8, 8)
        res = []
        for n2l in range(8):
            n2 = o8 + n2l
            z = wide(zt, pl.ds(pl.multiple_of(n2 * JZ, 8), JZ))
            res.append(_dot(_from_packed(t3[n2]), _split_rhs(z, 256 - 3 * JZ)))
        for r in range(4):
            t = _block_t(jnp.concatenate([res[n2l][8 * r:8 * r + 8] for n2l in range(8)], axis=0))
            for n1 in range(8):
                for g in range(NG):
                    yp[g, pl.ds(64 * (8 * r + n1) + o8, 8), :] = t[8 * n1:8 * n1 + 8, 128 * g:128 * (g + 1)]
        return carry

    lax.fori_loop(0, 8, st3_body, 0)

    dsk = [dsk_ref[g].astype(f32) for g in range(NG)]

    def ep_body(c, carry):
        r = pl.ds(pl.multiple_of(c * 64, 64), 64)
        for g in range(NG):
            yb = yp[g, r, :].astype(bf16).astype(f32)
            ud = (uf[g, r, :] * dsk[g]).astype(bf16).astype(f32)
            out_ref[r, pl.ds(D_MODEL + 128 * g, 128)] = (yb + ud).astype(bf16)
        _out_b_copy(out_ref, out_hbm, osems, c).start()
        return carry

    lax.fori_loop(0, 32, ep_body, 0)

    def ep_wait(c, carry):
        _out_b_copy(out_ref, out_hbm, osems, c).wait()
        return carry

    lax.fori_loop(0, 32, ep_wait, 0)


_SSM_SCRATCH = [
    pltpu.VMEM((4, 128, 128), f32),
    pltpu.VMEM((2, 32, 128, 128), f32),
    pltpu.VMEM((2, N_COARSE, 128, 128), f32),
    pltpu.VMEM((NG, L_SEQ + 8, 128), f32),
    pltpu.VMEM((NG, L_SEQ, 128), f32),
    pltpu.VMEM((64, JP // 2, 128), i32),
    pltpu.VMEM((64, 16, 256), i32),
    pltpu.VMEM((64, 128 * (3 if PASSES2 == 3 else 1)), i32),
    pltpu.VMEM((64, 128 * (3 if PASSES2 == 3 else 1)), i32),
    pltpu.VMEM((NG, 33 * 128, 128), f32),
    pltpu.VMEM((NG, 33 * 128, 128), f32),
    pltpu.VMEM((NG, 64 * JZ, 128), f32),
    pltpu.VMEM((NG, 64 * 32, 128), f32),
    pltpu.VMEM((33 * 128, 512), f32),
    pltpu.VMEM((2, 8, JP, 128), f32),
    pltpu.VMEM((2, 8, 32, 256), f32),
]


def _kernel(x_hbm, wqkv_hbm, wo_hbm, u_hbm, are_h, aim_h, bre_h, bim_h, cre_h, cim_h, ldt_ref, dsk_ref, out_hbm,
            xv, wv, wov, uv, pv, outv, sems, osems,
            wqT, wvT, k3, qT3, vT3, oT, bias, sS, mS, pS, lS, pmask, *ssm_scratch):
    in_copies = [pltpu.make_async_copy(src, dst, sems.at[k]) for k, (src, dst) in enumerate((
        (x_hbm, xv), (wqkv_hbm, wv), (wo_hbm, wov), (u_hbm, uv),
        (are_h, pv.at[0]), (aim_h, pv.at[1]), (bre_h, pv.at[2]), (bim_h, pv.at[3]),
        (cre_h, pv.at[4]), (cim_h, pv.at[5])))]
    for cp in in_copies:
        cp.start()
    (lam, tabF, tabC, kall, uf, t1, t3, f2, f2i, bsu, bsk, zt, yp, ys, tq1, tq3) = ssm_scratch
    _build_dft_tables(t1, t3, f2, f2i, tq1, tq3)
    for cp in in_copies[:3]:
        cp.wait()
    prm = tuple(pv.at[k] for k in range(6))

    def wait_ssm_inputs():
        for cp in in_copies[3:]:
            cp.wait()

    def host(body):
        item0 = body * BLK_PER_BODY
        _kgen_maybe_prep(item0, prm, ldt_ref, lam, tabF, tabC, kall)
        blks = [_KgenBlock(item0 + b, tabF, tabC, kall) for b in range(BLK_PER_BODY)]
        state = {"n": 0}

        def micro(zdep):
            b, nb = divmod(state["n"], 16)
            blks[b].step(nb, zdep)
            if nb == 15:
                blks[b].finish()
            state["n"] += 1

        return micro

    _attention_part(xv, wv, wov, outv, wqT, wvT, k3, qT3, vT3, oT, bias, sS, mS, pS, lS, pmask, host,
                    wait_ssm_inputs)
    out_a = pltpu.make_async_copy(outv.at[:, pl.ds(0, D_MODEL)], out_hbm.at[:, pl.ds(0, D_MODEL)], sems.at[10])
    out_a.start()
    _ssm_part(uv, prm, ldt_ref, dsk_ref, outv, out_hbm, osems, *ssm_scratch)
    out_a.wait()


@jax.jit
def pallas_concat_heads__sliding_block__ssm_conv_s4__prompt_kernel(
    A_x: jax.Array,
    A_wqkv: jax.Array,
    A_wo: jax.Array,
    B_u: jax.Array,
    B_A_re: jax.Array,
    B_A_im: jax.Array,
    B_B_re: jax.Array,
    B_B_im: jax.Array,
    B_C_re: jax.Array,
    B_C_im: jax.Array,
    B_log_dt: jax.Array,
    B_Dskip: jax.Array,
):
    x = A_x.reshape(S_LEN, D_MODEL)
    io_scratch = [
        pltpu.VMEM((S_LEN, D_MODEL), bf16),
        pltpu.VMEM((D_MODEL, 3 * D_MODEL), bf16),
        pltpu.VMEM((D_MODEL, D_MODEL), bf16),
        pltpu.VMEM((L_SEQ, D_MODEL), bf16),
        pltpu.VMEM((6, D_MODEL, 128), bf16),
        pltpu.VMEM((S_LEN, 2 * D_MODEL), bf16),
        pltpu.SemaphoreType.DMA((11,)),
        pltpu.SemaphoreType.DMA((32,)),
    ]
    scratch = [
        pltpu.VMEM((D_MODEL, D_MODEL), bf16),
        pltpu.VMEM((D_MODEL, D_MODEL), bf16),
        pltpu.VMEM((NG, S_LEN, 128), bf16),
        pltpu.VMEM((NQB, D_MODEL, QB), bf16),
        pltpu.VMEM((NQB, D_MODEL, QB), bf16),
        pltpu.VMEM((D_MODEL, QB), bf16),
        pltpu.VMEM((QB, QB), f32),
        pltpu.VMEM((N_HEADS, 2 * QB, QB), f32),
        pltpu.VMEM((N_HEADS, 1, QB), f32),
        pltpu.VMEM((N_HEADS, 2 * QB, QB), bf16),
        pltpu.VMEM((N_HEADS, 1, QB), f32),
        pltpu.VMEM((2, QB // 2, QB), i32),
    ]
    out = pl.pallas_call(
        _kernel,
        out_shape=jax.ShapeDtypeStruct((S_LEN, 2 * D_MODEL), bf16),
        in_specs=[pl.BlockSpec(memory_space=pl.ANY)] * 10 + [pl.BlockSpec(memory_space=pltpu.VMEM)] * 2,
        out_specs=pl.BlockSpec(memory_space=pl.ANY),
        scratch_shapes=io_scratch + scratch + _SSM_SCRATCH,
        compiler_params=pltpu.CompilerParams(vmem_limit_bytes=110 * 1024 * 1024),
    )(x, A_wqkv, A_wo, B_u.reshape(L_SEQ, D_MODEL), B_A_re, B_A_im, B_B_re, B_B_im, B_C_re, B_C_im,
      B_log_dt.reshape(NG, 1, 128), B_Dskip.reshape(NG, 1, 128))
    return out.reshape(1, S_LEN, 2 * D_MODEL)
```

```python
import functools
import math

import jax
import jax.numpy as jnp
from jax import lax
import jax.experimental.pallas as pl
import jax.experimental.pallas.tpu as pltpu

f32 = jnp.float32
bf16 = jnp.bfloat16
i32 = jnp.int32

S_LEN = 2048
D_MODEL = 512
N_HEADS = 32
D_HEAD = 16
WINDOW = 256
QB = 128
NQB = S_LEN // QB
NG = 4
NEG = -1e9


def _dot(a, b):
    return jnp.dot(a, b, preferred_element_type=f32)


def _dot_nt(a, b):
    return lax.dot_general(a, b, (((1,), (1,)), ((), ())), preferred_element_type=f32)


def _dot_tn(a, b):
    return lax.dot_general(a, b, (((0,), (0,)), ((), ())), preferred_element_type=f32)


def _attention_part(x_ref, wqkv_ref, wo_ref, out_ref, wqT, wvT, k3, qT3, vT3, oT, bias, pS, lS, pmask, host=None,
                    before_host=None):
    for (col0, dst) in ((0, wqT), (2 * D_MODEL, wvT)):
        for r in range(4):
            for c in range(4):
                blk = wqkv_ref[pl.ds(128 * r, 128), pl.ds(col0 + 128 * c, 128)].astype(f32)
                dst[pl.ds(128 * c, 128), pl.ds(128 * r, 128)] = blk.T.astype(bf16)

    rr = lax.broadcasted_iota(i32, (QB, QB), 0)
    cc = lax.broadcasted_iota(i32, (QB, QB), 1)
    bias[...] = jnp.where(rr <= cc, 0.0, NEG).astype(f32)
    r2 = lax.broadcasted_iota(i32, (QB // 2, QB), 0) * 2
    c2 = lax.broadcasted_iota(i32, (QB // 2, QB), 1)
    mt = jnp.where(r2 > c2, 0xFFFF, 0) | jnp.where(r2 + 1 > c2, -65536, 0)
    pmask[0] = mt
    pmask[1] = ~mt

    wk = wqkv_ref[:, pl.ds(D_MODEL, D_MODEL)]

    def proj_body(i, c, hosting=False):
        if hosting:
            micro = host((i - PROJ_PLAIN) * PROJ_BLK, PROJ_BLK)
        r0 = pl.multiple_of(i * QB, QB)
        xb = x_ref[pl.ds(r0, QB), :]
        kf = _dot(xb, wk)
        qf = _dot_nt(wqT[...], xb)
        if hosting:
            for k in range(PROJ_BLK * 16 * SUB):
                src, v = (kf, k) if k < 64 else (qf, k - 64)
                zsrc = src[8 * (v % 16):8 * (v % 16) + 8, 128 * (v // 16):128 * (v // 16) + 128] if k < 64 \
                    else src[8 * v:8 * v + 8, :]
                micro(jnp.minimum(jnp.abs(zsrc), 0.0))
        kb = kf.astype(bf16)
        for g in range(NG):
            k3[g, pl.ds(r0, QB), :] = kb[:, 128 * g:128 * (g + 1)]
        qT3[i] = (qf * (D_HEAD ** -0.5 * math.log2(math.e))).astype(bf16)
        vT3[i] = _dot_nt(wvT[...], xb).astype(bf16)
        return c

    if host is None:
        lax.fori_loop(0, NQB, proj_body, 0)
    else:
        lax.fori_loop(0, PROJ_PLAIN, proj_body, 0)
        before_host()
        lax.fori_loop(PROJ_PLAIN, NQB, functools.partial(proj_body, hosting=True), 0)
    k3w, qT3w, vT3w, pSw = (r.bitcast(i32) for r in (k3, qT3, vT3, pS))

    def attend(i, nblk):
        R = QB * min(nblk, 2)

        def phase1(g, c):
            hosting = host is not None and nblk == 3
            if hosting:
                micro = host(PROJ_HOSTED + ((i - 2) * NG + g) * BLK_PER_BODY, BLK_PER_BODY)
            kr0 = pl.multiple_of((i - nblk + 1) * (QB // 2), QB // 2)
            for hh in range(8):
                h = 8 * g + hh
                qh = qT3w[i, pl.ds(64 * g + 8 * hh, 8), :]
                pieces = []
                if hh > 0:
                    pieces.append(jnp.zeros((8 * hh, QB), i32))
                pieces.append(qh)
                if hh < 7:
                    pieces.append(jnp.zeros((56 - 8 * hh, QB), i32))
                qsel = _from_packed(jnp.concatenate(pieces, axis=0))
                sb = [_dot(_from_packed(k3w[g, pl.ds(kr0 + 64 * j, 64), :]), qsel) for j in range(nblk)]
                if nblk == 3:
                    blocks = [sb[1], jnp.where(rr > cc, sb[0], sb[2])]
                elif nblk == 2:
                    blocks = [sb[0], sb[1] + bias[...]]
                else:
                    blocks = [sb[0] + bias[...]]
                if hosting:
                    nt = SUB * MICRO_PER_HEAD
                    for k in range(nt):
                        v = (k * 32) // nt
                        micro(jnp.minimum(jnp.abs(blocks[v % 2][8 * (v // 2):8 * (v // 2) + 8, :]), 0.0))
                m = blocks[0].max(axis=0, keepdims=True)
                for b in blocks[1:]:
                    m = jnp.maximum(m, b.max(axis=0, keepdims=True))
                l = None
                for j, b in enumerate(blocks):
                    p = jnp.exp2(b - m)
                    ps = p.sum(axis=0, keepdims=True)
                    l = ps if l is None else l + ps
                    pS[h, pl.ds(QB * j, QB), :] = p.astype(bf16)
                lS[h] = l
            return c

        lax.fori_loop(0, NG, phase1, 0)

        def phase3(g, c):
            for hh in range(8):
                h = 8 * g + hh
                dr = pl.ds(64 * g + 8 * hh, 8)
                if nblk == 3:
                    pg = pSw[h, pl.ds(64, 64), :]
                    rhs = jnp.concatenate([pg & pmask[0], pSw[h, pl.ds(0, 64), :], pg & pmask[1]], axis=0)
                else:
                    rhs = pSw[h, pl.ds(0, R // 2), :]
                lhs = jnp.concatenate([vT3w[i - nblk + 1 + j, dr, :] for j in range(nblk)], axis=1)
                o = _dot(_from_packed(lhs), _from_packed(rhs))
                oT[pl.ds(128 * g + 16 * hh, 16), :] = (o / lS[h]).astype(bf16)
            return c

        lax.fori_loop(0, NG, phase3, 0)
        r0 = pl.multiple_of(i * QB, QB)
        out_ref[pl.ds(r0, QB), pl.ds(0, D_MODEL)] = _dot_tn(oT[...], wo_ref[...]).astype(bf16)

    attend(0, 1)
    attend(1, 2)

    def attn_body(i, c):
        attend(i, 3)
        return c

    lax.fori_loop(2, NQB, attn_body, 0)


L_SEQ = 2048
M_FFT = 4096
NJ = 66
JP = 80
JZ = 72
PASSES2 = 3

_P1 = 1.5703125
_P2 = 4.837512969970703125e-4
_P3 = 7.54978995489188216e-8


def _sincos_poly(r):
    r2 = r * r
    s = r + r * r2 * (-1.6666654611e-1 + r2 * (8.3321608736e-3 + r2 * (-1.9515295891e-4)))
    c = 1.0 - 0.5 * r2 + r2 * r2 * (4.166664568298827e-2 + r2 * (-1.388731625493765e-3 + r2 * 2.443315711809948e-5))
    return s, c


def _quadrant_fix(q, s, c):
    swap = (q & 1) == 1
    sn = jnp.where(swap, c, s)
    cs = jnp.where(swap, s, c)
    sn = jnp.where((q & 2) == 2, -sn, sn)
    cs = jnp.where(((q + 1) & 2) == 2, -cs, cs)
    return cs, sn


def _cis(theta):
    qf = jnp.floor(theta * (2.0 / math.pi) + 0.5)
    r = theta - qf * _P1
    r = r - qf * _P2
    r = r - qf * _P3
    s, c = _sincos_poly(r)
    return _quadrant_fix(qf.astype(i32), s, c)


def _trig_int(m):
    q = (m + 512) >> 10
    r = (m - (q << 10)).astype(f32) * (2.0 * math.pi / M_FFT)
    s, c = _sincos_poly(r)
    return _quadrant_fix(q, s, c)


def _hi(x):
    return lax.bitcast_convert_type(lax.bitcast_convert_type(x, i32) & jnp.int32(-65536), f32)


def _to_packed(x_f32):
    return pltpu.bitcast(x_f32.astype(bf16), i32)


def _from_packed(x_i32):
    return pltpu.bitcast(x_i32, bf16)


def _plan_powers():
    direct = (1, 8, 64, 512)
    have, ops = set(), []

    def ensure(e):
        if e in have:
            return
        if e in direct:
            ops.append(("direct", e))
        elif e & (e - 1) == 0:
            ensure(e // 2)
            ops.append(("sq", e, e // 2))
        else:
            hb = 1 << (e.bit_length() - 1)
            ensure(hb)
            ensure(e - hb)
            ops.append(("mul", e, hb, e - hb))
        have.add(e)

    for s in (1, 2, 4, 8):
        for b in range(1, 8):
            ensure(s * b)
        for b in range(1, 8):
            ensure(8 * s * b)
    for e in (64, 128, 192, 256, 512, 1024, 2048):
        ensure(e)
    return ops


_POWER_PLAN = _plan_powers()
N_COARSE = 81
NA = 2
MICRO_PER_HEAD = 4
BLK_PER_BODY = MICRO_PER_HEAD // 2
SUB = 2
PROJ_PLAIN = 4
PROJ_BLK = 4
PROJ_HOSTED = (16 - PROJ_PLAIN) * PROJ_BLK


def _build_dft_tables(t1, t3, f2, f2i, tq1, tq3):
    ncol = 128 * (3 if PASSES2 == 3 else 1)
    row = lax.broadcasted_iota(i32, (128, ncol), 0)
    col = lax.broadcasted_iota(i32, (128, ncol), 1)
    p = col >> 7
    ci = col & 127
    po, k2 = row >> 6, row & 63
    pi_, n2 = ci >> 6, ci & 63
    c, s = _trig_int(((k2 * n2) & 63) << 6)
    for dst, sgn in ((f2, 1.0), (f2i, -1.0)):
        val = jnp.where(po == pi_, c, jnp.where(po == 0, sgn * s, -sgn * s))
        hi = val.astype(bf16).astype(f32)
        dst[...] = _to_packed(jnp.where(p == 1, val - hi, hi))

    r1 = lax.broadcasted_iota(i32, (JP, 128), 0)
    c1 = lax.broadcasted_iota(i32, (JP, 128), 1)
    k1_1 = r1 >> 1
    ca1, sa1 = _trig_int((k1_1 * ((c1 & 31) << 6)) & (M_FFT - 1))
    r3 = lax.broadcasted_iota(i32, (32, 256), 0)
    c3 = lax.broadcasted_iota(i32, (32, 256), 1)
    p3 = (c3 >= JZ).astype(i32) + (c3 >= 2 * JZ).astype(i32) + (c3 >= 3 * JZ).astype(i32)
    j3 = c3 - JZ * p3
    k1_3 = j3 >> 1
    ca3, sa3 = _trig_int((k1_3 * (r3 << 6)) & (M_FFT - 1))
    for b in range(8):
        tq1[0, b], tq1[1, b] = _trig_int(k1_1 * b)
        tq3[0, b], tq3[1, b] = _trig_int(k1_3 * b)

    def body(a, carry):
        pc1, ps1 = _trig_int(k1_1 * (8 * a))
        pc3, ps3 = _trig_int(k1_3 * (8 * a))
        for b in range(8):
            n2 = 8 * a + b
            bc, bs = _cmul((pc1, ps1), (tq1[0, b], tq1[1, b]))
            c, sn = _cmul((ca1, sa1), (bc, bs))
            val = jnp.where((r1 & 1) == 0, c, -sn)
            val = jnp.where((r1 < NJ) & (c1 < 96), val, 0.0)
            hi = val.astype(bf16).astype(f32)
            t1[n2] = _to_packed(jnp.where((c1 >> 5) == 1, val - hi, hi))
            bc, bs = _cmul((pc3, ps3), (tq3[0, b], tq3[1, b]))
            c, sn = _cmul((ca3, sa3), (bc, bs))
            val = jnp.where((j3 & 1) == 0, c, -sn)
            w = jnp.where((k1_3 == 0) | (k1_3 == 32), 1.0 / M_FFT, 2.0 / M_FFT)
            val = jnp.where((j3 < NJ) & (p3 < 3), val * w, 0.0)
            hi = val.astype(bf16).astype(f32)
            t3[n2] = _to_packed(jnp.where(p3 == 1, val - hi, hi))
        return carry

    lax.fori_loop(0, 8, body, 0)


def _cmul(a, b):
    return a[0] * b[0] - a[1] * b[1], a[0] * b[1] + a[1] * b[0]


def _kgen_prep(g, prm_refs, ldt_ref, lam, tabF, tabC, kall):
    are, aim, bre, bim, cre, cim = prm_refs
    r0 = pl.multiple_of(g * 128, 128)
    dt = jnp.exp(ldt_ref[g].astype(f32)).astype(bf16).astype(f32)

    def tr(ref):
        return ref[pl.ds(r0, 128), :].astype(f32).T

    dbr = tr(bre) * dt
    dbi = tr(bim) * dt
    cr_, ci_ = tr(cre), tr(cim)
    lam[0] = tr(are) * dt
    lam[1] = tr(aim) * dt
    lam[2] = cr_ * dbr - ci_ * dbi
    lam[3] = cr_ * dbi + ci_ * dbr

    CH = 16

    def tab_body(ch, carry):
        rows = pl.ds(pl.multiple_of(ch * CH, CH), CH)
        lr, li = lam[0, rows, :], lam[1, rows, :]
        cc = (lam[2, rows, :], lam[3, rows, :])
        W = {}
        for op in _POWER_PLAN:
            if op[0] == "direct":
                e = float(op[1])
                mag = jnp.exp(lr * e)
                c, s = _cis(li * e)
                W[op[1]] = (mag * c, mag * s)
            elif op[0] == "sq":
                a, b = W[op[2]]
                W[op[1]] = (a * a - b * b, (a + a) * b)
            else:
                W[op[1]] = _cmul(W[op[2]], W[op[3]])
        for si, s in enumerate((1, 2, 4, 8)):
            for b in range(1, 8):
                tabF[0, 8 * si + b, rows, :] = W[s * b][0]
                tabF[1, 8 * si + b, rows, :] = W[s * b][1]

        def put(idx, v):
            tabC[0, idx, rows, :] = v[0]
            tabC[1, idx, rows, :] = v[1]

        base = cc
        for p in range(4):
            if p > 0:
                base = _cmul(cc, W[64 * p])
            put(8 * p, base)
            for i in range(1, 8):
                put(8 * p + i, _cmul(base, W[8 * i]))
        for si, s in ((1, 2), (2, 4), (3, 8)):
            base = _cmul(cc, W[128 * s])
            for p in range(2):
                if p == 1:
                    base = _cmul(base, W[64 * s])
                o = 32 + 16 * (si - 1) + 8 * p
                put(o, base)
                for i in range(1, 8):
                    put(o + i, _cmul(base, W[8 * s * i]))
        put(80, _cmul(cc, W[2048]))
        return carry

    lax.fori_loop(0, 128 // CH, tab_body, 0)
    kall[g, pl.ds(L_SEQ, 1), :] = jnp.sum(tabC[0, 80], axis=0, keepdims=True)


NBLK_G = 80 // NA


class _KgenBlock:
    def __init__(self, item, tabF, tabC, kall):
        self.tabF, self.tabC, self.kall = tabF, tabC, kall
        self.g = item // NBLK_G
        kk = item - self.g * NBLK_G
        nb0 = 32 // NA
        nbs = 16 // NA
        si = jnp.where(kk < nb0, 0, 1 + (kk - nb0) // nbs)
        self.a0 = jnp.where(kk < nb0, NA * kk, 16 + NA * ((kk - nb0) % nbs))
        self.step_ = jnp.left_shift(1, si)
        self.fbase = 8 * si
        self.kk = kk
        self.acc = [[None] * 8 for _ in range(NA)]

    def step(self, nb, zdep=None, bs=range(8)):
        tabF, tabC, acc = self.tabF, self.tabC, self.acc
        rows = pl.ds(8 * nb, 8)
        cr = [tabC[0, NA * self.kk + a, rows, :] for a in range(NA)]
        ci = [tabC[1, NA * self.kk + a, rows, :] for a in range(NA)]
        if zdep is not None:
            cr = [c + zdep for c in cr]
            ci = [c + zdep for c in ci]
        for b in bs:
            if b > 0:
                fr = tabF[0, self.fbase + b, rows, :]
                fi = tabF[1, self.fbase + b, rows, :]
            for a in range(NA):
                term = cr[a] if b == 0 else cr[a] * fr - ci[a] * fi
                acc[a][b] = term if nb == 0 else acc[a][b] + term

    def finish(self):
        for a in range(NA):
            for b in range(8):
                row = self.step_ * (8 * (self.a0 + a) + b)
                self.kall[self.g, pl.ds(row, 1), :] = jnp.sum(self.acc[a][b], axis=0, keepdims=True)


def _kgen_maybe_prep(item, prm_refs, ldt_ref, lam, tabF, tabC, kall):
    g = item // NBLK_G

    @pl.when(item - g * NBLK_G == 0)
    def _():
        _kgen_prep(g, prm_refs, ldt_ref, lam, tabF, tabC, kall)


def _kgen_item(item, tabF, tabC, kall):
    blk = _KgenBlock(item, tabF, tabC, kall)
    for nb in range(16):
        blk.step(nb)
    blk.finish()


def _split_rhs(x, extra_zero_rows=0):
    xh = _hi(x)
    pieces = [xh, xh, x - xh]
    if extra_zero_rows:
        pieces.append(jnp.zeros((extra_zero_rows, x.shape[1]), f32))
    return jnp.concatenate(pieces, axis=0).astype(bf16)


def _block_t(v):
    return jnp.swapaxes(v.reshape(8, 8, v.shape[1]), 0, 1).reshape(64, v.shape[1])


def _round_off(n2, s):
    q = n2 // s
    rem = n2 - q * s
    up = (rem * 2 > s) | ((rem * 2 == s) & ((q & 1) == 1))
    return (q + up.astype(i32)) * s


def _out_b_copy(outv, out_hbm, osems, c):
    r = pl.ds(pl.multiple_of(c * 64, 64), 64)
    cols = pl.ds(D_MODEL, D_MODEL)
    return pltpu.make_async_copy(outv.at[r, cols], out_hbm.at[r, cols], osems.at[c])


def _ssm_part(u_ref, prm_refs, ldt_ref, dsk_ref, out_ref, out_hbm, osems,
              lam, tabF, tabC, kall, uf, t1, t3, f2, f2i, bsu, bsk, zt, yp, ys, tq1, tq3):
    for g in range(NG):
        uf[g] = u_ref[:, pl.ds(128 * g, 128)].astype(f32)

    def kg(item, c):
        _kgen_maybe_prep(item, prm_refs, ldt_ref, lam, tabF, tabC, kall)
        _kgen_item(item, tabF, tabC, kall)
        return c

    n_hosted = PROJ_HOSTED + (NQB - 2) * NG * BLK_PER_BODY
    if n_hosted < NG * NBLK_G:
        lax.fori_loop(n_hosted, NG * NBLK_G, kg, 0)

    def st1_body(o, carry):
        o8 = pl.multiple_of(o * 8, 8)
        tu = []
        for r in range(4):
            v = jnp.concatenate([
                jnp.concatenate([uf[g, pl.ds(64 * (8 * r + n1) + o8, 8), :] for g in range(NG)], axis=1)
                for n1 in range(8)], axis=0)
            tu.append(_block_t(v))
        for name in ("u", "k"):
            res = []
            for n2l in range(8):
                n2 = o8 + n2l
                if name == "u":
                    x = jnp.concatenate([tu[r][8 * n2l:8 * n2l + 8] for r in range(4)], axis=0)
                else:
                    o2, o4, o8_ = 256 + _round_off(n2, 2), 512 + _round_off(n2, 4), 1024 + _round_off(n2, 8)
                    x = jnp.concatenate([jnp.concatenate([
                        kall[g, pl.ds(n2, 4, stride=64), :],
                        kall[g, pl.ds(o2, 4, stride=64), :],
                        kall[g, pl.ds(o4, 8, stride=64), :],
                        kall[g, pl.ds(o8_, 16, stride=64), :]], axis=0) for g in range(NG)], axis=1)
                res.append(_dot(_from_packed(t1[n2]), _split_rhs(x, 32)))
            dst = bsu if name == "u" else bsk
            for q in range(9):
                t = _block_t(jnp.concatenate([res[n2l][8 * q:8 * q + 8] for n2l in range(8)], axis=0))
                for jj in range(8):
                    if 8 * q + jj < NJ:
                        for g in range(NG):
                            dst[g, pl.ds(64 * (8 * q + jj) + o8, 8), :] = t[8 * jj:8 * jj + 8, 128 * g:128 * (g + 1)]
        return carry

    lax.fori_loop(0, 8, st1_body, 0)

    def prep(x):
        if PASSES2 == 3:
            return _split_rhs(x)
        return x.astype(bf16)

    def wide(ref, rows):
        return jnp.concatenate([ref[g, rows, :] for g in range(NG)], axis=1)

    def k1f_body(k1, carry):
        lf = _from_packed(f2[...])
        r = pl.ds(pl.multiple_of(k1 * 128, 128), 128)
        xu = _dot(lf, prep(wide(bsu, r)))
        xk = _dot(lf, prep(wide(bsk, r)))
        ur, ui, kr, ki = xu[:64], xu[64:], xk[:64], xk[64:]
        ys[r, :] = jnp.concatenate([ur * kr - ui * ki, ur * ki + ui * kr], axis=0)
        return carry

    lax.fori_loop(0, 33, k1f_body, 0, unroll=3)

    def put_zt(blocks, q):
        for o in range(8):
            t = _block_t(jnp.concatenate([b[8 * o:8 * o + 8] for b in blocks], axis=0))
            for n2l in range(8):
                for g in range(NG):
                    zt[g, pl.ds((8 * o + n2l) * JZ + 8 * q, 8), :] = t[8 * n2l:8 * n2l + 8, 128 * g:128 * (g + 1)]

    def k1i_body(q, carry):
        li = _from_packed(f2i[...])
        blocks = []
        for a in range(4):
            z = _dot(li, prep(ys[pl.ds(pl.multiple_of((4 * q + a) * 128, 128), 128), :]))
            blocks += [z[:64], z[64:]]
        put_zt(blocks, q)
        return carry

    lax.fori_loop(0, 8, k1i_body, 0)
    z = _dot(_from_packed(f2i[...]), prep(ys[pl.ds(32 * 128, 128), :]))
    put_zt([z[:64], z[64:]] + [jnp.zeros((64, 128 * NG), f32)] * 6, 8)

    def st3_body(o, carry):
        o8 = pl.multiple_of(o * 8, 8)
        res = []
        for n2l in range(8):
            n2 = o8 + n2l
            z = wide(zt, pl.ds(pl.multiple_of(n2 * JZ, 8), JZ))
            res.append(_dot(_from_packed(t3[n2]), _split_rhs(z, 256 - 3 * JZ)))
        for r in range(4):
            t = _block_t(jnp.concatenate([res[n2l][8 * r:8 * r + 8] for n2l in range(8)], axis=0))
            for n1 in range(8):
                for g in range(NG):
                    yp[g, pl.ds(64 * (8 * r + n1) + o8, 8), :] = t[8 * n1:8 * n1 + 8, 128 * g:128 * (g + 1)]
        return carry

    lax.fori_loop(0, 8, st3_body, 0)

    dsk = [dsk_ref[g].astype(f32) for g in range(NG)]

    def ep_body(c, carry):
        r = pl.ds(pl.multiple_of(c * 64, 64), 64)
        for g in range(NG):
            yb = yp[g, r, :].astype(bf16).astype(f32)
            ud = (uf[g, r, :] * dsk[g]).astype(bf16).astype(f32)
            out_ref[r, pl.ds(D_MODEL + 128 * g, 128)] = (yb + ud).astype(bf16)
        _out_b_copy(out_ref, out_hbm, osems, c).start()
        return carry

    lax.fori_loop(0, 32, ep_body, 0)

    def ep_wait(c, carry):
        _out_b_copy(out_ref, out_hbm, osems, c).wait()
        return carry

    lax.fori_loop(0, 32, ep_wait, 0)


_SSM_SCRATCH = [
    pltpu.VMEM((4, 128, 128), f32),
    pltpu.VMEM((2, 32, 128, 128), f32),
    pltpu.VMEM((2, N_COARSE, 128, 128), f32),
    pltpu.VMEM((NG, L_SEQ + 8, 128), f32),
    pltpu.VMEM((NG, L_SEQ, 128), f32),
    pltpu.VMEM((64, JP // 2, 128), i32),
    pltpu.VMEM((64, 16, 256), i32),
    pltpu.VMEM((64, 128 * (3 if PASSES2 == 3 else 1)), i32),
    pltpu.VMEM((64, 128 * (3 if PASSES2 == 3 else 1)), i32),
    pltpu.VMEM((NG, 33 * 128, 128), f32),
    pltpu.VMEM((NG, 33 * 128, 128), f32),
    pltpu.VMEM((NG, 64 * JZ, 128), f32),
    pltpu.VMEM((NG, 64 * 32, 128), f32),
    pltpu.VMEM((33 * 128, 512), f32),
    pltpu.VMEM((2, 8, JP, 128), f32),
    pltpu.VMEM((2, 8, 32, 256), f32),
]


def _kernel(x_hbm, wqkv_hbm, wo_hbm, u_hbm, are_h, aim_h, bre_h, bim_h, cre_h, cim_h, ldt_ref, dsk_ref, out_hbm,
            xv, wv, wov, uv, pv, outv, sems, osems,
            wqT, wvT, k3, qT3, vT3, oT, bias, pS, lS, pmask, *ssm_scratch):
    in_copies = [pltpu.make_async_copy(src, dst, sems.at[k]) for k, (src, dst) in enumerate((
        (x_hbm, xv), (wqkv_hbm, wv), (wo_hbm, wov), (u_hbm, uv),
        (are_h, pv.at[0]), (aim_h, pv.at[1]), (bre_h, pv.at[2]), (bim_h, pv.at[3]),
        (cre_h, pv.at[4]), (cim_h, pv.at[5])))]
    for cp in in_copies:
        cp.start()
    (lam, tabF, tabC, kall, uf, t1, t3, f2, f2i, bsu, bsk, zt, yp, ys, tq1, tq3) = ssm_scratch
    _build_dft_tables(t1, t3, f2, f2i, tq1, tq3)
    for cp in in_copies[:3]:
        cp.wait()
    prm = tuple(pv.at[k] for k in range(6))

    def wait_ssm_inputs():
        for cp in in_copies[3:]:
            cp.wait()

    def host(item0, nblk_):
        _kgen_maybe_prep(item0, prm, ldt_ref, lam, tabF, tabC, kall)
        blks = [_KgenBlock(item0 + b, tabF, tabC, kall) for b in range(nblk_)]
        state = {"n": 0}

        def micro(zdep):
            n, part = divmod(state["n"], SUB)
            b, nb = divmod(n, 16)
            w = 8 // SUB
            blks[b].step(nb, zdep, range(w * part, w * part + w))
            if nb == 15 and part == SUB - 1:
                blks[b].finish()
            state["n"] += 1

        return micro

    _attention_part(xv, wv, wov, outv, wqT, wvT, k3, qT3, vT3, oT, bias, pS, lS, pmask, host,
                    wait_ssm_inputs)
    out_a = pltpu.make_async_copy(outv.at[:, pl.ds(0, D_MODEL)], out_hbm.at[:, pl.ds(0, D_MODEL)], sems.at[10])
    out_a.start()
    _ssm_part(uv, prm, ldt_ref, dsk_ref, outv, out_hbm, osems, *ssm_scratch)
    out_a.wait()


@jax.jit
def pallas_concat_heads__sliding_block__ssm_conv_s4__prompt_kernel(
    A_x: jax.Array,
    A_wqkv: jax.Array,
    A_wo: jax.Array,
    B_u: jax.Array,
    B_A_re: jax.Array,
    B_A_im: jax.Array,
    B_B_re: jax.Array,
    B_B_im: jax.Array,
    B_C_re: jax.Array,
    B_C_im: jax.Array,
    B_log_dt: jax.Array,
    B_Dskip: jax.Array,
):
    x = A_x.reshape(S_LEN, D_MODEL)
    io_scratch = [
        pltpu.VMEM((S_LEN, D_MODEL), bf16),
        pltpu.VMEM((D_MODEL, 3 * D_MODEL), bf16),
        pltpu.VMEM((D_MODEL, D_MODEL), bf16),
        pltpu.VMEM((L_SEQ, D_MODEL), bf16),
        pltpu.VMEM((6, D_MODEL, 128), bf16),
        pltpu.VMEM((S_LEN, 2 * D_MODEL), bf16),
        pltpu.SemaphoreType.DMA((11,)),
        pltpu.SemaphoreType.DMA((32,)),
    ]
    scratch = [
        pltpu.VMEM((D_MODEL, D_MODEL), bf16),
        pltpu.VMEM((D_MODEL, D_MODEL), bf16),
        pltpu.VMEM((NG, S_LEN, 128), bf16),
        pltpu.VMEM((NQB, D_MODEL, QB), bf16),
        pltpu.VMEM((NQB, D_MODEL, QB), bf16),
        pltpu.VMEM((D_MODEL, QB), bf16),
        pltpu.VMEM((QB, QB), f32),
        pltpu.VMEM((N_HEADS, 2 * QB, QB), bf16),
        pltpu.VMEM((N_HEADS, 1, QB), f32),
        pltpu.VMEM((2, QB // 2, QB), i32),
    ]
    out = pl.pallas_call(
        _kernel,
        out_shape=jax.ShapeDtypeStruct((S_LEN, 2 * D_MODEL), bf16),
        in_specs=[pl.BlockSpec(memory_space=pl.ANY)] * 10 + [pl.BlockSpec(memory_space=pltpu.VMEM)] * 2,
        out_specs=pl.BlockSpec(memory_space=pl.ANY),
        scratch_shapes=io_scratch + scratch + _SSM_SCRATCH,
        compiler_params=pltpu.CompilerParams(vmem_limit_bytes=110 * 1024 * 1024),
    )(x, A_wqkv, A_wo, B_u.reshape(L_SEQ, D_MODEL), B_A_re, B_A_im, B_B_re, B_B_im, B_C_re, B_C_im,
      B_log_dt.reshape(NG, 1, 128), B_Dskip.reshape(NG, 1, 128))
    return out.reshape(1, S_LEN, 2 * D_MODEL)
```
